```python
import os as _os
_os.environ.setdefault("JAX_PLATFORMS", "cpu")
import jax
import jax.numpy as jnp

def _softmax(x, axis=-1):
    return jax.nn.softmax(x, axis=axis)
def _gelu(x):
    return jax.nn.gelu(x, approximate=True)
def _silu(x):
    return jax.nn.silu(x)
def _sigmoid(x):
    return jax.nn.sigmoid(x)
def _layernorm(x, axis=-1, eps=1e-5):
    m = jnp.mean(x, axis=axis, keepdims=True)
    v = jnp.var(x, axis=axis, keepdims=True)
    return (x - m) / jnp.sqrt(v + eps)
def _scatter_add(tgt, idx, src, axis=0):
    return tgt.at[idx].add(src)
def _segment_sum(src, seg, n):
    return jax.ops.segment_sum(src, seg, n)
class _Rng:
    def __init__(self, key):
        self._k = key
    def _next(self):
        self._k, sub = jax.random.split(self._k)
        return sub
    def normal(self, shape):
        return jax.random.normal(self._next(), shape, dtype=jnp.bfloat16)
    def randint(self, lo, hi, shape):
        return jax.random.randint(self._next(), shape, lo, hi, dtype=jnp.int32)
    def uniform(self, shape, lo=0.0, hi=1.0):
        return jax.random.uniform(self._next(), shape, jnp.bfloat16, lo, hi)
    def permutation(self, n):
        return jax.random.permutation(self._next(), n)


kernel_name = 'interleave_layers__mha_block__dense_activation_gelu__prompt'

def setup_inputs():
    _rng = _Rng(jax.random.key(int.from_bytes(__import__("os").urandom(4), "little")))
    _w = (lambda a: (lambda t: t.astype(jnp.bfloat16) if jnp.issubdtype(t.dtype, jnp.floating) else t)(jnp.asarray(a)))
    def _A_setup():
        B, S, D, H = 1, 2048, 512, 32
        return {
            "x": _w((lambda *s: _rng.normal(s) * 0.05)(B, S, D)),
            "wqkv": _w((lambda *s: _rng.normal(s) * 0.05)(D, 3 * D)),
            "wo": _w((lambda *s: _rng.normal(s) * 0.05)(D, D)),
        }
    _A_in = _A_setup()

    def _B_setup():
        B, S, D, F = 1, 2048, 512, 1792
        return {
            "x": _w((lambda *s: _rng.normal(s) * 0.05)(B, S, D)),
            "w1": _w((lambda *s: _rng.normal(s) * 0.4)(D, F) * (D ** -0.5)),
            "b1": _w((lambda *s: _rng.normal(s) * 0.4)(F) * 0.01),
            "w2": _w((lambda *s: _rng.normal(s) * 0.4)(F, D) * (F ** -0.5)),
            "b2": _w((lambda *s: _rng.normal(s) * 0.4)(D) * 0.01),
        }
    _B_in = _B_setup()

    return {
        "A_x": _A_in["x"],
        "A_wqkv": _A_in["wqkv"],
        "A_wo": _A_in["wo"],
        "B_x": _B_in["x"],
        "B_w1": _B_in["w1"],
        "B_b1": _B_in["b1"],
        "B_w2": _B_in["w2"],
        "B_b2": _B_in["b2"],
    }

def reference(A_x, A_wqkv, A_wo, B_x, B_w1, B_b1, B_w2, B_b2):
    def _A_ref(x, wqkv, wo):
        B, S, D = x.shape
        H = 32
        Dh = D // H
        qkv = (lambda x, *d: x.transpose(*d))((x @ wqkv).reshape(B, S, 3, H, Dh), 2, 0, 3, 1, 4)
        q, k, v = qkv[0], qkv[1], qkv[2]
        scores = jnp.einsum("bhqd,bhkd->bhqk", q, k) * (Dh ** -0.5)
        p = _softmax(scores, axis=-1)
        o = jnp.einsum("bhqk,bhkd->bhqd", p, v)
        return (lambda x, *d: x.transpose(*d))(o, 0, 2, 1, 3).reshape(B, S, D) @ wo

    def _B_ref(x, w1, b1, w2, b2):
        h = jnp.einsum("bsd,df->bsf", x, w1) + b1
        h = _gelu(h)
        return jnp.einsum("bsf,fd->bsd", h, w2) + b2

    x = A_x
    x = x + _A_ref(_layernorm(x, axis=-1), A_wqkv, A_wo)
    x = x + _B_ref(_layernorm(x, axis=-1), B_w1, B_b1, B_w2, B_b2)
    x = x + _A_ref(_layernorm(x, axis=-1), A_wqkv, A_wo)
    x = x + _B_ref(_layernorm(x, axis=-1), B_w1, B_b1, B_w2, B_b2)
    return x
```

```python
import jax
import jax.numpy as jnp
import jax.experimental.pallas as pl
import jax.experimental.pallas.tpu as pltpu

S, D, H, DH, F = 2048, 512, 32, 16, 1792
NG = H // 2
N_LAYERS = 2
EPS = 1e-5
LOG2E = 1.4426950408889634
SCALE = DH ** -0.5
MAGIC = 12582912.0

TX = 512
TA = 256
TA2 = 1024
TM = 512
TS = 256
TQ = 1024
TK = 128
PAIRS = 1
NC = S // 128
ND = D // 128
NX = S // TX
QS = 40

SAFE_LOG2 = 100.0

bf16 = jnp.bfloat16
f32 = jnp.float32
i32 = jnp.int32
i8 = jnp.int8
NT = (((1,), (1,)), ((), ()))
TN = (((0,), (0,)), ((), ()))


def _layernorm(x):
    m = jnp.mean(x, axis=-1, keepdims=True)
    xc = x - m
    v = jnp.mean(xc * xc, axis=-1, keepdims=True)
    return xc * jax.lax.rsqrt(v + EPS)


def _gelu(x):
    c = 0.7978845608028654
    return 0.5 * x * (1.0 + jnp.tanh(c * (x + 0.044715 * (x * x * x))))


def _bits(t):
    return pltpu.bitcast(t, i32)


def _kernel(x_hbm, wqkv_hbm, wo_hbm, w1_hbm, b1_ref, w2_hbm, b2_ref, o_hbm,
            xb, wqkv, wo, w1, w2, sems,
            xs, xns, wqT, wvT, tmp, kf, kmx, qT, vT, kl, qw, cs, al, oT, p_c, acc_c, l_c):

    def x_copy(t):
        return pltpu.make_async_copy(x_hbm.at[pl.ds(t * TX, TX), :],
                                     xb.at[pl.ds(t * TX, TX), :], sems.at[t])

    def wqkv_copy(j):
        return pltpu.make_async_copy(wqkv_hbm.at[:, pl.ds(j * D, D)], wqkv.at[j], sems.at[NX + j])

    late = [pltpu.make_async_copy(src, dst, sems.at[NX + 3 + j])
            for j, (src, dst) in enumerate(((wo_hbm, wo), (w1_hbm, w1), (w2_hbm, w2)))]

    def out_copy(t):
        r0 = pl.multiple_of(t * TM, TM)
        return pltpu.make_async_copy(xb.at[pl.ds(r0, TM), :], o_hbm.at[pl.ds(r0, TM), :],
                                     sems.at[NX + 6 + t])

    x_copy(0).start()
    wqkv_copy(1).start()
    for t in range(1, NX):
        x_copy(t).start()
    wqkv_copy(0).start()
    wqkv_copy(2).start()

    def wide(ref, rows=slice(None)):
        return jnp.concatenate([ref[j, rows, :] for j in range(ND)], axis=1)

    def ln_store(x, r0, n):
        xn = _layernorm(x).astype(bf16)
        for j in range(ND):
            xns[j, pl.ds(r0, n), :] = xn[:, j * 128:(j + 1) * 128]
        return xn

    def k_proj(xn, r0, n):
        k = jnp.dot(xn, wqkv[1], preferred_element_type=f32)
        kf[pl.ds(r0, n), :] = k
        return jnp.max(jnp.abs(k).reshape(n // 8, 8, D), axis=0)

    kmax8 = jnp.zeros((8, D), f32)
    for t in range(NX):
        x_copy(t).wait()
        if t == 0:
            wqkv_copy(1).wait()
            for cp in late:
                cp.start()
        if t == NX - 1:
            wqkv_copy(0).wait()
            wqkv_copy(2).wait()
            wv_t = wqkv[2].T
            wq_t = wqkv[0].T.astype(f32)
            for j in range(ND):
                wvT[j] = wv_t[:, j * 128:(j + 1) * 128]
                tmp[j] = wq_t[:, j * 128:(j + 1) * 128]
            for j in range(ND):
                for o in range(4):
                    for d2 in range(DH // 2):
                        r = o * 128 + d2 * 16
                        wqT[j, r:r + 16, :] = jnp.concatenate(
                            [tmp[j, pl.ds(o * 128 + 2 * d2 + e, 8, stride=DH), :]
                             for e in range(2)], axis=0).astype(bf16)
        for u in range(TX // TA):
            r0 = t * TX + u * TA
            x = xb[r0:r0 + TA, :].astype(f32)
            xs[r0:r0 + TA, :] = x
            kmax8 = jnp.maximum(kmax8, k_proj(ln_store(x, r0, TA), r0, TA))
    kmx[...] = kmax8

    def layer(li, carry):
        kmax = jnp.maximum(jnp.max(kmx[...], axis=0, keepdims=True), 1e-30)
        beta = 127.0 / kmax
        tmp[0] = jnp.broadcast_to(kmax, (128, D)).T
        for o in range(4):
            for d in range(DH):
                r = o * 128 + d * 8
                tmp[1, r:r + 8, :] = tmp[0, pl.ds(o * 128 + d, 8, stride=DH), :]
        beta8 = jnp.broadcast_to(beta, (8, D))

        def k_limbs(r0, gg):
            seg = (jax.lax.broadcasted_iota(i32, (8, 128), 1) // DH) % 4
            y = kf[pl.ds(r0, 32), gg * 128:(gg + 1) * 128].reshape(4, 8, 128) \
                * beta8[:, gg * 128:(gg + 1) * 128]
            t0 = y + MAGIC
            te = (y - (t0 - MAGIC)) + MAGIC / 16
            t1 = y + MAGIC * 16
            y0, e1, y1 = [pltpu.bitcast(_bits(a).reshape(32, 128).astype(i8), i32)
                          for a in (t0, te, t1)]

            def rolled(a, k):
                return a if k == 0 else pltpu.roll(a, (DH * k) % 128, 1)
            ry0 = {k: rolled(y0, k) for k in range(-3, 2)}
            re1 = {k: rolled(e1, k) for k in range(-1, 3)}
            ry1 = {k: rolled(y1, k) for k in range(0, 4)}
            for r in range(4):
                out = jnp.where(seg < 2,
                                jnp.where(seg == 0, ry0[0 - r], ry0[1 - r]),
                                jnp.where(seg == 2, re1[2 - r], ry1[3 - r]))
                kl[gg * 4 + r, pl.ds(r0, 32), :] = pltpu.bitcast(out, i8)

        def q_limbs(ct, o, k):
            r = o * 128 + k * 32
            x = qT[ct, r:r + 32, :].reshape(4, 8, 128) * al[ct, o * 8:(o + 1) * 8, :]
            t0 = x + MAGIC
            u = _bits(x + MAGIC * 2)
            v = _bits(t0) - u
            x1 = _bits(x + MAGIC * 16)
            e = _bits((x - (t0 - MAGIC)) + MAGIC / 16)
            for j, a in enumerate((u, v, x1, e)):
                word = pltpu.pack_elementwise([a[b] for b in range(4)], packed_dtype=i8)
                r = (4 * j + k) * QS + o * 8
                qw[ct, r:r + 8, :] = pltpu.bitcast(word, i32)

        def qproj(t, bound):
            for cc in range(TA2 // 128):
                ct = t * (TA2 // 128) + cc
                r0 = pl.multiple_of(ct * 128, 128)
                q = jax.lax.dot_general(wide(wqT), wide(xns, pl.ds(r0, 128)), NT,
                                        preferred_element_type=f32) * tmp[1]
                qT[ct] = q
                aq = jnp.abs(q).reshape(4, DH, 8, 128)
                amax = jnp.maximum(jnp.max(aq, axis=1), 1e-30).reshape(H, 128)
                al[ct] = 254.0 / amax
                cs[ct] = amax * (SCALE * LOG2E / (254.0 * 127.0))
                bound = jnp.maximum(bound, jnp.max(jnp.sum(aq, axis=1), axis=0))
                for rb in range(4):
                    for gg in range(4):
                        k_limbs(pl.multiple_of(r0 + rb * 32, 32), gg)
            return bound
        bound = jax.lax.fori_loop(0, S // TA2, qproj, jnp.zeros((8, 128), f32))
        safe = jnp.max(bound) * (SCALE * LOG2E) < SAFE_LOG2

        def vproj(t, _):
            for cc in range(TA2 // 128):
                ct = t * (TA2 // 128) + cc
                r0 = pl.multiple_of(ct * 128, 128)
                xn = wide(xns, pl.ds(r0, 128))
                for o in range(4):
                    rows = slice(o * 128, (o + 1) * 128)
                    v = jax.lax.dot_general(wide(wvT, rows), xn, NT,
                                            preferred_element_type=f32)
                    vT[ct, rows, :] = v.astype(bf16)
                    for k in range(4):
                        q_limbs(ct, o, k)
            return 0
        jax.lax.fori_loop(0, S // TA2, vproj, 0)

        @pl.when(safe)
        def _fast():
            nq = S // TQ
            nk = S // TK
            cq = TQ // 128

            def row0(h):
                return h * DH if isinstance(h, int) else pl.multiple_of(h * DH, DH)

            def pv(h, kc, pb, acc):
                return acc + jnp.dot(vT[kc, pl.ds(row0(h), DH), :], pb,
                                     preferred_element_type=f32)

            def finish(h, q0, acc, ls):
                lsum = jnp.sum(ls, axis=0, keepdims=True)
                oT[pl.ds(row0(h), DH), pl.ds(q0, TQ)] = (acc / lsum).astype(bf16)

            def head_of(g, b):
                return (g // 4) * 8 + 4 * b + g % 4

            p_c[...] = jnp.zeros(p_c.shape, bf16)
            acc_c[...] = jnp.zeros(acc_c.shape, f32)
            l_c[...] = jnp.ones(l_c.shape, f32)

            def body(i, _):
                ph, pq0 = head_of(jnp.maximum(i * PAIRS - 1, 0), 1), (nq - 1) * TQ
                pb, acc, pls = p_c[...], acc_c[0], l_c[...]
                zero = jnp.zeros((DH, TQ), i32)
                for gi in range(PAIRS):
                    g = i * PAIRS + gi
                    for b in range(2):
                        h = head_of(g, b)
                        for qt in range(nq):
                            words = jnp.concatenate(
                                [qw[qt * cq + j, pl.ds(h, DH, stride=QS), :] for j in range(cq)],
                                axis=1)
                            w = pltpu.bitcast(jnp.concatenate(
                                [words, zero] if b == 0 else [zero, words], axis=0), i8)
                            c = jnp.concatenate(
                                [cs[qt * cq + j, pl.ds(h, 1), :] for j in range(cq)], axis=1)
                            ls = None
                            for kc in range(nk):
                                s = jnp.dot(kl[g, pl.ds(kc * TK, TK), :], w,
                                            preferred_element_type=i32)
                                if kc == 0:
                                    finish(ph, pq0, pv(ph, nk - 1, pb, acc), pls)
                                    acc = acc_c[1]
                                else:
                                    acc = pv(h, kc - 1, pb, acc)
                                p = jnp.exp2(s.astype(f32) * c)
                                psum = jnp.sum(p.reshape(TK // 8, 8, TQ), axis=0)
                                ls = psum if ls is None else ls + psum
                                pb = p.astype(bf16)
                            ph, pq0, pls = h, qt * TQ, ls
                p_c[...] = pb
                acc_c[0] = acc
                l_c[...] = pls
                return 0
            jax.lax.fori_loop(0, NG // PAIRS, body, 0)
            finish(H - 1, (nq - 1) * TQ, pv(H - 1, nk - 1, p_c[...], acc_c[0]), l_c[...])

        @pl.when(jnp.logical_not(safe))
        def _slow():
            def qraw(ct, _):
                r0 = pl.multiple_of(ct * 128, 128)
                qT[ct] = jax.lax.dot_general(wide(wqT), wide(xns, pl.ds(r0, 128)), NT,
                                             preferred_element_type=f32)
                return 0
            jax.lax.fori_loop(0, NC, qraw, 0)

            def body(i, _):
                h = i // NC
                ct = i % NC
                q0 = pl.multiple_of(ct * 128, 128)
                g0 = pl.multiple_of((h // 8) * 128, 128)
                r0 = pl.multiple_of(h * DH, DH)
                qh = qT[ct, pl.ds(g0 + h % 8, DH, stride=8), :]
                row = jax.lax.broadcasted_iota(i32, (128, 128), 0)
                w = jnp.where(row // DH == h % 8, jnp.concatenate([qh] * 8, axis=0), 0.0)
                kb = kf[:, pl.ds(g0, 128)].astype(bf16)
                s = jnp.dot(kb, w.astype(bf16), preferred_element_type=f32) * SCALE
                m = jnp.max(s, axis=0, keepdims=True)
                p = jnp.exp(s - m)
                lsum = jnp.sum(p, axis=0, keepdims=True)
                vh = jnp.concatenate([vT[j, pl.ds(r0, DH), :] for j in range(NC)], axis=1)
                acc = jnp.dot(vh, p.astype(bf16), preferred_element_type=f32)
                oT[pl.ds(r0, DH), pl.ds(q0, 128)] = (acc / lsum).astype(bf16)
                return 0
            jax.lax.fori_loop(0, H * NC, body, 0)

        def ffn(t, last):
            ns = TM // TS
            rs = [pl.multiple_of(t * TM + u * TS, TS) for u in range(ns)]
            b1 = b1_ref[...].astype(f32)
            b2 = b2_ref[...].astype(f32)
            x1 = [xs[pl.ds(r, TS), :] + jax.lax.dot_general(
                oT[:, pl.ds(r, TS)], wo[...], TN, preferred_element_type=f32) for r in rs]
            hh = [_gelu(jnp.dot(_layernorm(x).astype(bf16), w1[...],
                                preferred_element_type=f32) + b1).astype(bf16) for x in x1]
            x2 = [x + jnp.dot(g, w2[...], preferred_element_type=f32) + b2
                  for x, g in zip(x1, hh)]
            if last:
                for r, x in zip(rs, x2):
                    xb[pl.ds(r, TS), :] = x.astype(bf16)
                out_copy(t).start()
            else:
                km = kmx[...]
                for r, x in zip(rs, x2):
                    xs[pl.ds(r, TS), :] = x
                    km = jnp.maximum(km, k_proj(ln_store(x, r, TS), r, TS))
                kmx[...] = km
            return 0

        @pl.when(li == 0)
        def _():
            for cp in late:
                cp.wait()

        @pl.when(li < N_LAYERS - 1)
        def _():
            kmx[...] = jnp.zeros(kmx.shape, f32)
            jax.lax.fori_loop(0, S // TM, lambda t, _: ffn(t, False), 0)

        @pl.when(li == N_LAYERS - 1)
        def _():
            jax.lax.fori_loop(0, S // TM, lambda t, _: ffn(t, True), 0)
        return carry

    jax.lax.fori_loop(0, N_LAYERS, layer, 0)
    for t in range(S // TM):
        out_copy(t).wait()


@jax.jit
def pallas_interleave_layers__mha_block__dense_activation_gelu__prompt_kernel(
    A_x: jax.Array,
    A_wqkv: jax.Array,
    A_wo: jax.Array,
    B_x: jax.Array,
    B_w1: jax.Array,
    B_b1: jax.Array,
    B_w2: jax.Array,
    B_b2: jax.Array,
):
    del B_x
    hbm = pl.BlockSpec(memory_space=pl.ANY)
    vmem = pl.BlockSpec(memory_space=pltpu.VMEM)
    out = pl.pallas_call(
        _kernel,
        out_shape=jax.ShapeDtypeStruct((S, D), A_x.dtype),
        in_specs=[hbm, hbm, hbm, hbm, vmem, hbm, vmem],
        out_specs=hbm,
        scratch_shapes=[
            pltpu.VMEM((S, D), bf16),
            pltpu.VMEM((3, D, D), bf16),
            pltpu.VMEM((D, D), bf16),
            pltpu.VMEM((D, F), bf16),
            pltpu.VMEM((F, D), bf16),
            pltpu.SemaphoreType.DMA((NX + 6 + S // TM,)),
            pltpu.VMEM((S, D), f32),
            pltpu.VMEM((ND, S, 128), bf16),
            pltpu.VMEM((ND, D, 128), bf16),
            pltpu.VMEM((ND, D, 128), bf16),
            pltpu.VMEM((ND, D, 128), f32),
            pltpu.VMEM((S, D), f32),
            pltpu.VMEM((8, D), f32),
            pltpu.VMEM((NC, D, 128), f32),
            pltpu.VMEM((NC, D, 128), bf16),
            pltpu.VMEM((NG, S, 128), i8),
            pltpu.VMEM((NC, DH * QS, 128), i32),
            pltpu.VMEM((NC, H, 128), f32),
            pltpu.VMEM((NC, H, 128), f32),
            pltpu.VMEM((D, S), bf16),
            pltpu.VMEM((TK, TQ), bf16),
            pltpu.VMEM((2, DH, TQ), f32),
            pltpu.VMEM((8, TQ), f32),
        ],
        compiler_params=pltpu.CompilerParams(vmem_limit_bytes=100 * 1024 * 1024),
    )(A_x.reshape(S, D), A_wqkv, A_wo, B_w1, B_b1.reshape(1, F), B_w2, B_b2.reshape(1, D))
    return out.reshape(1, S, D)
```

```python
import jax
import jax.numpy as jnp
import jax.experimental.pallas as pl
import jax.experimental.pallas.tpu as pltpu

S, D, H, DH, F = 2048, 512, 32, 16, 1792
N_LAYERS = 2
EPS = 1e-5
LOG2E = 1.4426950408889634
SCALE = DH ** -0.5
MAGIC = 12582912.0

NG = H // 2
NC = S // 128
ND = D // 128
X_CHUNKS = ((0, 256), (256, 256), (512, 512), (1024, 1024))
NX = len(X_CHUNKS)
TA = 256
W_AT = 5
TA2 = 1024
TM = 512
TS = 256
TQ = 1024
TK = 128
HS = 24
QS = 40

SAFE_LOG2 = 64.0
WV_MIN, WV_MAX = 2.0 ** -20, 2.0 ** 20

bf16 = jnp.bfloat16
f32 = jnp.float32
i32 = jnp.int32
i8 = jnp.int8
NT = (((1,), (1,)), ((), ()))
TN = (((0,), (0,)), ((), ()))


def _layernorm(x):
    m = jnp.mean(x, axis=-1, keepdims=True)
    xc = x - m
    v = jnp.mean(xc * xc, axis=-1, keepdims=True)
    return xc * jax.lax.rsqrt(v + EPS)


def _gelu(x):
    c = 0.7978845608028654
    return 0.5 * x * (1.0 + jnp.tanh(c * (x + 0.044715 * (x * x * x))))


def _bits(t):
    return pltpu.bitcast(t, i32)


def _wide(ref, rows=slice(None)):
    return jnp.concatenate([ref[j, rows, :] for j in range(ref.shape[0])], axis=1)


def _aligned(i, n):
    return i if isinstance(i, int) else pl.multiple_of(i, n)


def _kernel(x_hbm, wqkv_hbm, wo_hbm, w1_hbm, b1_hbm, w2_hbm, b2_hbm, o_hbm,
            xb, wqkv, wo, w1, w2, sems,
            xs, xns, wqT, wvT, tmp, kf, kmx, qT, vT, kl, qw, cs, al, oT, oN,
            p_c, acc_c, l_c, k_c, v_c, c_c, b1v, b2v, b1f, b2f):

    def x_copy(c):
        r0, n = X_CHUNKS[c]
        return pltpu.make_async_copy(x_hbm.at[pl.ds(r0, n), :], xb.at[pl.ds(r0, n), :],
                                     sems.at[c])

    def wqkv_copy(j):
        return pltpu.make_async_copy(wqkv_hbm.at[:, pl.ds(j * D, D)], wqkv.at[j],
                                     sems.at[NX + j])

    late = [pltpu.make_async_copy(src, dst, sems.at[NX + 3 + j])
            for j, (src, dst) in enumerate(
                ((wo_hbm, wo), (w1_hbm, w1), (w2_hbm, w2), (b1_hbm, b1v), (b2_hbm, b2v)))]

    def out_copy(u):
        r0 = _aligned(u * TS, TS)
        return pltpu.make_async_copy(xb.at[pl.ds(r0, TS), :], o_hbm.at[pl.ds(r0, TS), :],
                                     sems.at[NX + 8 + u])

    x_copy(0).start()
    wqkv_copy(1).start()
    for c in range(1, NX):
        x_copy(c).start()
    wqkv_copy(0).start()
    wqkv_copy(2).start()
    for cp in late:
        cp.start()

    for ct in range(NC):
        for j in range(DH):
            qw[ct, j * QS + H:(j + 1) * QS, :] = jnp.zeros((QS - H, 128), i32)
        qw[ct, DH * QS:, :] = jnp.zeros((QS, 128), i32)
        qT[ct, D:, :] = jnp.zeros((8, 128), f32)
    for j in range(ND):
        for h in range(H):
            tmp[j, h * HS + DH:(h + 1) * HS, :] = jnp.zeros((HS - DH, 128), f32)
        tmp[j, H * HS:, :] = jnp.zeros((HS, 128), f32)

    def ln_store(x, r0, n):
        xn = _layernorm(x).astype(bf16)
        for j in range(ND):
            xns[j, pl.ds(r0, n), :] = xn[:, j * 128:(j + 1) * 128]
        return xn

    def k_proj(xn, r0, n):
        k = jnp.dot(xn, wqkv[1], preferred_element_type=f32)
        kf[pl.ds(r0, n), :] = k
        return jnp.max(jnp.abs(k).reshape(n // 8, 8, D), axis=0)

    def first_ln(u):
        x = xb[u * TA:(u + 1) * TA, :].astype(f32)
        xs[u * TA:(u + 1) * TA, :] = x
        ln_store(x, u * TA, TA)

    def w_transposes():
        wv_t = wqkv[2].T
        wq_t = wqkv[0].T.astype(f32)
        for j in range(ND):
            wvT[j] = wv_t[:, j * 128:(j + 1) * 128]
            for h in range(H):
                tmp[j, h * HS:h * HS + DH, :] = wq_t[h * DH:(h + 1) * DH, j * 128:(j + 1) * 128]
        for j in range(ND):
            for o in range(4):
                for d2 in range(DH // 2):
                    r = o * 128 + d2 * 16
                    wqT[j, r:r + 16, :] = jnp.concatenate(
                        [tmp[j, pl.ds(o * 8 * HS + 2 * d2 + e, 8, stride=HS), :]
                         for e in range(2)], axis=0).astype(bf16)
        wv_max = jnp.max(jnp.abs(wqkv[2].astype(f32)))
        return (wv_max >= WV_MIN) & (wv_max <= WV_MAX)

    x_copy(0).wait()
    first_ln(0)
    kmax8 = jnp.zeros((8, D), f32)
    starts = {r0 // TA: c for c, (r0, _) in enumerate(X_CHUNKS)}
    for u in range(S // TA):
        if u == 0:
            wqkv_copy(1).wait()
        if u + 1 in starts:
            x_copy(starts[u + 1]).wait()
        if u == W_AT:
            wqkv_copy(0).wait()
            wqkv_copy(2).wait()
        kmax8 = jnp.maximum(kmax8, k_proj(_wide(xns, slice(u * TA, (u + 1) * TA)), u * TA, TA))
        if u + 1 < S // TA:
            first_ln(u + 1)
        if u == W_AT:
            v_ok = w_transposes()
    kmx[...] = kmax8

    def layer(li, carry):
        def k_stats():
            kmax = jnp.maximum(jnp.max(kmx[...], axis=0, keepdims=True), 1e-30)
            kc = jnp.broadcast_to(kmax, (128, D)).T
            for h in range(H):
                tmp[0, h * HS:h * HS + DH, :] = kc[h * DH:(h + 1) * DH]
            for o in range(4):
                for d in range(DH):
                    r = o * 128 + d * 8
                    tmp[1, r:r + 8, :] = tmp[0, pl.ds(o * 8 * HS + d, 8, stride=HS), :]
            return jnp.broadcast_to(127.0 / kmax, (8, D))

        def k_limbs(r0, gg, beta8):
            seg = (jax.lax.broadcasted_iota(i32, (8, 128), 1) // DH) % 4
            y = kf[pl.ds(r0, 32), gg * 128:(gg + 1) * 128].reshape(4, 8, 128) \
                * beta8[:, gg * 128:(gg + 1) * 128]
            t0 = y + MAGIC
            te = (y - (t0 - MAGIC)) + MAGIC / 16
            t1 = y + MAGIC * 16
            y0, ey, y1 = [pltpu.bitcast(_bits(a).reshape(32, 128).astype(i8), i32)
                          for a in (t0, te, t1)]

            def rolled(a, k):
                return a if k == 0 else pltpu.roll(a, (DH * k) % 128, 1)
            ry0 = {k: rolled(y0, k) for k in range(-3, 2)}
            rey = {k: rolled(ey, k) for k in range(-1, 3)}
            ry1 = {k: rolled(y1, k) for k in range(0, 4)}
            for r in range(4):
                out = jnp.where(seg < 2,
                                jnp.where(seg == 0, ry0[0 - r], ry0[1 - r]),
                                jnp.where(seg == 2, rey[2 - r], ry1[3 - r]))
                kl[gg * 4 + r, pl.ds(r0, 32), :] = pltpu.bitcast(out, i8)

        def q_limbs(ct, o, k):
            r = o * 128 + k * 32
            x = qT[ct, r:r + 32, :].reshape(4, 8, 128) * al[ct, o * 8:(o + 1) * 8, :]
            t0 = x + MAGIC
            u = _bits(x + MAGIC * 2)
            v = _bits(t0) - u
            x1 = _bits(x + MAGIC * 16)
            ex = _bits((x - (t0 - MAGIC)) + MAGIC / 16)
            for j, a in enumerate((u, v, x1, ex)):
                word = pltpu.pack_elementwise([a[b] for b in range(4)], packed_dtype=i8)
                r = (4 * j + k) * QS + o * 8
                qw[ct, r:r + 8, :] = pltpu.bitcast(word, i32)

        def qproj(t, bound):
            beta8 = k_stats()
            for cc in range(TA2 // 128):
                ct = t * (TA2 // 128) + cc
                r0 = pl.multiple_of(ct * 128, 128)
                q = jax.lax.dot_general(_wide(wqT), _wide(xns, pl.ds(r0, 128)), NT,
                                        preferred_element_type=f32) * tmp[1, 0:D, :]
                qT[ct, 0:D, :] = q
                aq = jnp.abs(q).reshape(4, DH, 8, 128)
                amax = jnp.maximum(jnp.max(aq, axis=1), 1e-30).reshape(H, 128)
                al[ct] = 254.0 / amax
                cs[ct] = amax * (SCALE * LOG2E / (254.0 * 127.0))
                bound = jnp.maximum(bound, jnp.max(jnp.sum(aq, axis=1), axis=0))
                for rb in range(4):
                    for gg in range(4):
                        k_limbs(pl.multiple_of(r0 + rb * 32, 32), gg, beta8)
            return bound
        bound = jax.lax.fori_loop(0, S // TA2, qproj, jnp.zeros((8, 128), f32))

        def vproj(t, _):
            p_c[...] = jnp.zeros(p_c.shape, bf16)
            acc_c[...] = jnp.zeros(acc_c.shape, f32)
            l_c[...] = jnp.ones(l_c.shape, f32)
            v_c[1, S // TK - 1] = jnp.zeros((8, 128), i32)
            for cc in range(TA2 // 128):
                ct = t * (TA2 // 128) + cc
                r0 = pl.multiple_of(ct * 128, 128)
                xn = _wide(xns, pl.ds(r0, 128))
                for o in range(4):
                    rows = slice(o * 128, (o + 1) * 128)
                    v = jax.lax.dot_general(_wide(wvT, rows), xn, NT,
                                            preferred_element_type=f32)
                    vT[ct, rows, :] = v.astype(bf16)
                    for k in range(4):
                        q_limbs(ct, o, k)
            return jnp.max(bound)
        bmax = jax.lax.fori_loop(0, S // TA2, vproj, jnp.float32(0))
        safe = (bmax * (SCALE * LOG2E) < SAFE_LOG2) & v_ok

        def o_transpose(t):
            on = oT[:, pl.ds(_aligned(t * TM, TM), TS)].T
            for j in range(ND):
                oN[j] = on[:, j * 128:(j + 1) * 128]

        @pl.when(safe)
        def _fast():
            nq = S // TQ
            nk = S // TK
            cq = TQ // 128

            def head_of(g, b):
                return ((g >> 2) << 3) + 4 * b + (g & 3)

            def pv(v, pb, acc):
                return acc + jnp.dot(pltpu.bitcast(v, bf16), pb, preferred_element_type=f32)

            def finish(h, q0, acc, ls):
                lsum = jnp.sum(ls, axis=0, keepdims=True)
                r = pl.reciprocal(lsum, approx=True)
                r = r * (2.0 - lsum * r)
                oT[pl.ds(_aligned(h * DH, DH), DH), pl.ds(q0, TQ)] = (acc * r).astype(bf16)

            def body(g, _):
                ph, pq0 = head_of(jnp.maximum(g - 1, 0), 1), (nq - 1) * TQ
                pb, acc, pls, pv_last = p_c[...], acc_c[0], l_c[...], v_c[1, nk - 1]
                kg = pltpu.bitcast(kl[g], i32)
                k_c[0] = kg
                k_c[1] = pltpu.roll(kg, 64, 1)
                for b in range(2):
                    h = head_of(g, b)
                    for kc in range(nk):
                        v_c[b, kc] = pltpu.bitcast(
                            vT[kc, pl.ds(_aligned(h * DH, DH), DH), :], i32)
                    for j in range(NC):
                        c_c[b, :, j * 128:(j + 1) * 128] = jnp.broadcast_to(
                            cs[j, pl.ds(h, 1), :], (8, 128))
                zero = jnp.zeros((DH, TQ), i32)
                for qt in range(nq):
                    for b in range(2):
                        h = head_of(g, b)
                        words = jnp.concatenate(
                            [qw[qt * cq + j, pl.ds(h, DH, stride=QS), :] for j in range(cq)],
                            axis=1)
                        w = pltpu.bitcast(jnp.concatenate([words, zero], axis=0), i8)
                        c = c_c[b, :, qt * TQ:(qt + 1) * TQ]
                        ls = None
                        for kc in range(nk):
                            kk = k_c[b, kc * (TK // 4):(kc + 1) * (TK // 4), :]
                            s = jnp.dot(pltpu.bitcast(kk, i8), w, preferred_element_type=i32)
                            if kc == 0:
                                finish(ph, pq0, pv(pv_last, pb, acc), pls)
                                acc = acc_c[1]
                            else:
                                acc = pv(v_c[b, kc - 1], pb, acc)
                            p = jnp.exp2(s.astype(f32).reshape(TK // 8, 8, TQ) * c)
                            psum = jnp.sum(p, axis=0)
                            ls = psum if ls is None else ls + psum
                            pb = p.reshape(TK, TQ).astype(bf16)
                        ph, pq0, pls, pv_last = h, qt * TQ, ls, v_c[b, nk - 1]
                p_c[...] = pb
                acc_c[0] = acc
                l_c[...] = pls
                return 0
            jax.lax.fori_loop(0, NG, body, 0)
            o_transpose(0)
            finish(H - 1, (nq - 1) * TQ, pv(v_c[1, nk - 1], p_c[...], acc_c[0]), l_c[...])

        @pl.when(jnp.logical_not(safe))
        def _slow():
            def qraw(ct, _):
                r0 = pl.multiple_of(ct * 128, 128)
                qT[ct, 0:D, :] = jax.lax.dot_general(
                    _wide(wqT), _wide(xns, pl.ds(r0, 128)), NT, preferred_element_type=f32)
                return 0
            jax.lax.fori_loop(0, NC, qraw, 0)

            def body(i, _):
                h = i // NC
                ct = i % NC
                q0 = pl.multiple_of(ct * 128, 128)
                g0 = pl.multiple_of((h // 8) * 128, 128)
                r0 = pl.multiple_of(h * DH, DH)
                qh = qT[ct, pl.ds(g0 + h % 8, DH, stride=8), :]
                row = jax.lax.broadcasted_iota(i32, (128, 128), 0)
                w = jnp.where(row // DH == h % 8, jnp.concatenate([qh] * 8, axis=0), 0.0)
                kb = kf[:, pl.ds(g0, 128)].astype(bf16)
                s = jnp.dot(kb, w.astype(bf16), preferred_element_type=f32) * SCALE
                m = jnp.max(s, axis=0, keepdims=True)
                p = jnp.exp(s - m)
                lsum = jnp.sum(p, axis=0, keepdims=True)
                acc = jnp.dot(_wide(vT, pl.ds(r0, DH)), p.astype(bf16),
                              preferred_element_type=f32)
                oT[pl.ds(r0, DH), pl.ds(q0, 128)] = (acc / lsum).astype(bf16)
                return 0
            jax.lax.fori_loop(0, H * NC, body, 0)
            o_transpose(0)

        def ffn(t, last):
            ns = TM // TS
            rs = [pl.multiple_of(t * TM + u * TS, TS) for u in range(ns)]
            b1 = b1f[...]
            b2 = b2f[...]
            x1 = [xs[pl.ds(rs[0], TS), :] + jnp.dot(_wide(oN), wo[...],
                                                    preferred_element_type=f32)]
            x1 += [xs[pl.ds(r, TS), :] + jax.lax.dot_general(
                oT[:, pl.ds(r, TS)], wo[...], TN, preferred_element_type=f32) for r in rs[1:]]
            o_transpose(jnp.minimum(t + 1, S // TM - 1))
            hh = [_gelu(jnp.dot(_layernorm(x).astype(bf16), w1[...],
                                preferred_element_type=f32) + b1).astype(bf16) for x in x1]
            x2 = []
            for u, (r, x, g) in enumerate(zip(rs, x1, hh)):
                x = x + jnp.dot(g, w2[...], preferred_element_type=f32) + b2
                if last:
                    xb[pl.ds(r, TS), :] = x.astype(bf16)
                    out_copy(t * ns + u).start()
                else:
                    xs[pl.ds(r, TS), :] = x
                    x2.append(x)
            if not last:
                km = kmx[...]
                for r, x in zip(rs, x2):
                    km = jnp.maximum(km, k_proj(ln_store(x, r, TS), r, TS))
                kmx[...] = km
            return 0

        @pl.when(li == 0)
        def _():
            for cp in late:
                cp.wait()
            b1f[...] = b1v[...].astype(f32).reshape(1, F)
            b2f[...] = b2v[...].astype(f32).reshape(1, D)

        @pl.when(li < N_LAYERS - 1)
        def _():
            kmx[...] = jnp.zeros(kmx.shape, f32)
            jax.lax.fori_loop(0, S // TM, lambda t, _: ffn(t, False), 0)

        @pl.when(li == N_LAYERS - 1)
        def _():
            jax.lax.fori_loop(0, S // TM, lambda t, _: ffn(t, True), 0)
        return carry

    jax.lax.fori_loop(0, N_LAYERS, layer, 0)
    for u in range(S // TS):
        out_copy(u).wait()


@jax.jit
def pallas_interleave_layers__mha_block__dense_activation_gelu__prompt_kernel(
    A_x: jax.Array,
    A_wqkv: jax.Array,
    A_wo: jax.Array,
    B_x: jax.Array,
    B_w1: jax.Array,
    B_b1: jax.Array,
    B_w2: jax.Array,
    B_b2: jax.Array,
):
    del B_x
    hbm = pl.BlockSpec(memory_space=pl.ANY)
    out = pl.pallas_call(
        _kernel,
        out_shape=jax.ShapeDtypeStruct((S, D), A_x.dtype),
        in_specs=[hbm] * 7,
        out_specs=hbm,
        scratch_shapes=[
            pltpu.VMEM((S, D), bf16),
            pltpu.VMEM((3, D, D), bf16),
            pltpu.VMEM((D, D), bf16),
            pltpu.VMEM((D, F), bf16),
            pltpu.VMEM((F, D), bf16),
            pltpu.SemaphoreType.DMA((NX + 8 + S // TS,)),
            pltpu.VMEM((S, D), f32),
            pltpu.VMEM((ND, S, 128), bf16),
            pltpu.VMEM((ND, D, 128), bf16),
            pltpu.VMEM((ND, D, 128), bf16),
            pltpu.VMEM((ND, (H + 1) * HS, 128), f32),
            pltpu.VMEM((S, D), f32),
            pltpu.VMEM((8, D), f32),
            pltpu.VMEM((NC, D + 8, 128), f32),
            pltpu.VMEM((NC, D, 128), bf16),
            pltpu.VMEM((NG, S, 128), i8),
            pltpu.VMEM((NC, (DH + 1) * QS, 128), i32),
            pltpu.VMEM((NC, H, 128), f32),
            pltpu.VMEM((NC, H, 128), f32),
            pltpu.VMEM((D, S), bf16),
            pltpu.VMEM((ND, TS, 128), bf16),
            pltpu.VMEM((TK, TQ), bf16),
            pltpu.VMEM((2, DH, TQ), f32),
            pltpu.VMEM((8, TQ), f32),
            pltpu.VMEM((2, S // 4, 128), i32),
            pltpu.VMEM((2, NC, 8, 128), i32),
            pltpu.VMEM((2, 8, S), f32),
            pltpu.VMEM((F,), bf16),
            pltpu.VMEM((D,), bf16),
            pltpu.VMEM((1, F), f32),
            pltpu.VMEM((1, D), f32),
        ],
        compiler_params=pltpu.CompilerParams(vmem_limit_bytes=100 * 1024 * 1024),
    )(A_x.reshape(S, D), A_wqkv, A_wo, B_w1, B_b1, B_w2, B_b2)
    return out.reshape(1, S, D)
```

```python
import jax
import jax.numpy as jnp
import jax.experimental.pallas as pl
import jax.experimental.pallas.tpu as pltpu

S, D, H, DH, F = 2048, 512, 32, 16, 1792
N_LAYERS = 2
EPS = 1e-5
LOG2E = 1.4426950408889634
SCALE = DH ** -0.5
MAGIC = 12582912.0

SIGN_BYTES = 0x80808080 - 2 ** 32

NG = H // 2
NC = S // 128
ND = D // 128
X_CHUNKS = ((0, 256), (256, 256), (512, 512), (1024, 1024))
NX = len(X_CHUNKS)
TA = 256
W_AT = 5
TA2 = 1024
TM = 512
TS = 256
TQ = 1024
TK = 128
HS = 24
QS = 40

SAFE_LOG2 = 64.0
WV_MIN, WV_MAX = 2.0 ** -20, 2.0 ** 20

bf16 = jnp.bfloat16
f32 = jnp.float32
i32 = jnp.int32
i8 = jnp.int8
NT = (((1,), (1,)), ((), ()))
TN = (((0,), (0,)), ((), ()))


def _layernorm(x):
    m = jnp.mean(x, axis=-1, keepdims=True)
    xc = x - m
    v = jnp.mean(xc * xc, axis=-1, keepdims=True)
    return xc * jax.lax.rsqrt(v + EPS)


def _gelu(x):
    c = 0.7978845608028654
    return 0.5 * x * (1.0 + jnp.tanh(c * (x + 0.044715 * (x * x * x))))


def _bits(t):
    return pltpu.bitcast(t, i32)


PACKS = ((0, 256), (1, 128), (4, 128), (-4, 16 * 256 + 128))
BIG = 2.0 ** 31 + 2.0 ** 21


def _pack_consts(e, off):
    return [(BIG - 2.0 ** 23 - 257 * off - extra) * 2.0 ** e
            for extra in (0, 2 ** 16 - ((150 + e) << 7))]


def _pack_rounded(x, e, sub):
    def pair(lo, hi256, c):
        return _bits(((hi256 + BIG * 2.0 ** e) - c) + lo)
    return pair(x[0], x[1], sub[0]) + (pair(x[2], x[3], sub[1]) << 16)


def _wide(ref, rows=slice(None)):
    return jnp.concatenate([ref[j, rows, :] for j in range(ref.shape[0])], axis=1)


def _aligned(i, n):
    return i if isinstance(i, int) else pl.multiple_of(i, n)


def _kernel(x_hbm, wqkv_hbm, wo_hbm, w1_hbm, b1_hbm, w2_hbm, b2_hbm, o_hbm,
            xb, wqkv, wo, w1, w2, sems,
            xs, xns, wqT, wvT, tmp, kf, kmx, qT, vT, kl, qw, cs, al, oT, oN,
            p_c, acc_c, l_c, k_c, v_c, c_c, cst, b1v, b2v, b1f, b2f):

    def x_copy(c):
        r0, n = X_CHUNKS[c]
        return pltpu.make_async_copy(x_hbm.at[pl.ds(r0, n), :], xb.at[pl.ds(r0, n), :],
                                     sems.at[c])

    def wqkv_copy(j):
        return pltpu.make_async_copy(wqkv_hbm.at[:, pl.ds(j * D, D)], wqkv.at[j],
                                     sems.at[NX + j])

    late = [pltpu.make_async_copy(src, dst, sems.at[NX + 3 + j])
            for j, (src, dst) in enumerate(
                ((wo_hbm, wo), (w1_hbm, w1), (w2_hbm, w2), (b1_hbm, b1v), (b2_hbm, b2v)))]

    def out_copy(u):
        r0 = _aligned(u * TS, TS)
        return pltpu.make_async_copy(xb.at[pl.ds(r0, TS), :], o_hbm.at[pl.ds(r0, TS), :],
                                     sems.at[NX + 8 + u])

    x_copy(0).start()
    wqkv_copy(1).start()
    for c in range(1, NX):
        x_copy(c).start()
    wqkv_copy(0).start()
    wqkv_copy(2).start()
    for cp in late:
        cp.start()

    for i, (e, off) in enumerate(PACKS):
        for j, c in enumerate(_pack_consts(e, off)):
            cst[2 * i + j] = jnp.full((8, 128), c, f32)

    for ct in range(NC):
        for j in range(DH):
            qw[ct, j * QS + H:(j + 1) * QS, :] = jnp.zeros((QS - H, 128), i32)
        qw[ct, DH * QS:, :] = jnp.zeros((QS, 128), i32)
        qT[ct, D:, :] = jnp.zeros((8, 128), f32)
    for j in range(ND):
        for h in range(H):
            tmp[j, h * HS + DH:(h + 1) * HS, :] = jnp.zeros((HS - DH, 128), f32)
        tmp[j, H * HS:, :] = jnp.zeros((HS, 128), f32)

    def ln_store(x, r0, n):
        xn = _layernorm(x).astype(bf16)
        for j in range(ND):
            xns[j, pl.ds(r0, n), :] = xn[:, j * 128:(j + 1) * 128]
        return xn

    def k_proj(xn, r0, n):
        k = jnp.dot(xn, wqkv[1], preferred_element_type=f32)
        kf[pl.ds(r0, n), :] = k
        return jnp.max(jnp.abs(k).reshape(n // 8, 8, D), axis=0)

    def first_ln(u):
        ln_store(xb[u * TA:(u + 1) * TA, :].astype(f32), u * TA, TA)

    def w_transposes():
        wvT[...] = pltpu.bitcast(wqkv[2].T, i32)
        wq_t = wqkv[0].T.astype(f32)
        for j in range(ND):
            for h in range(H):
                tmp[j, h * HS:h * HS + DH, :] = wq_t[h * DH:(h + 1) * DH, j * 128:(j + 1) * 128]
        for j in range(ND):
            for o in range(4):
                for d2 in range(DH // 2):
                    r = o * 64 + d2 * 8
                    wqT[r:r + 8, j * 128:(j + 1) * 128] = pltpu.bitcast(jnp.concatenate(
                        [tmp[j, pl.ds(o * 8 * HS + 2 * d2 + e, 8, stride=HS), :]
                         for e in range(2)], axis=0).astype(bf16), i32)
        wv_max = jnp.max(jnp.abs(wqkv[2].astype(f32)))
        return (wv_max >= WV_MIN) & (wv_max <= WV_MAX)

    x_copy(0).wait()
    first_ln(0)
    kmax8 = jnp.zeros((8, D), f32)
    starts = {r0 // TA: c for c, (r0, _) in enumerate(X_CHUNKS)}
    for u in range(S // TA):
        if u == 0:
            wqkv_copy(1).wait()
        if u + 1 in starts:
            x_copy(starts[u + 1]).wait()
        if u == W_AT:
            wqkv_copy(0).wait()
            wqkv_copy(2).wait()
        kmax8 = jnp.maximum(kmax8, k_proj(_wide(xns, slice(u * TA, (u + 1) * TA)), u * TA, TA))
        if u + 1 < S // TA:
            first_ln(u + 1)
        if u == W_AT:
            v_ok = w_transposes()
    kmx[...] = kmax8

    def layer(li, carry):
        def k_stats():
            kmax = jnp.maximum(jnp.max(kmx[...], axis=0, keepdims=True), 1e-30)
            kc = jnp.broadcast_to(kmax, (128, D)).T
            for h in range(H):
                tmp[0, h * HS:h * HS + DH, :] = kc[h * DH:(h + 1) * DH]
            for o in range(4):
                for d in range(DH):
                    r = o * 128 + d * 8
                    tmp[1, r:r + 8, :] = tmp[0, pl.ds(o * 8 * HS + d, 8, stride=HS), :]
            return jnp.broadcast_to(127.0 / kmax, (8, D))

        def k_limbs(r0, gg, beta8):
            seg = (jax.lax.broadcasted_iota(i32, (8, 128), 1) // DH) % 4
            y = kf[pl.ds(r0, 32), gg * 128:(gg + 1) * 128].reshape(4, 8, 128) \
                * beta8[:, gg * 128:(gg + 1) * 128]
            t0 = _bits(y + MAGIC)
            te = _bits(y + MAGIC / 16) - (t0 << 4)
            t1 = _bits(y + MAGIC * 16)
            y0, ey, y1 = [pltpu.bitcast(a.reshape(32, 128).astype(i8), i32)
                          for a in (t0, te, t1)]

            def rolled(a, k):
                return a if k == 0 else pltpu.roll(a, (DH * k) % 128, 1)
            ry0 = {k: rolled(y0, k) for k in range(-3, 2)}
            rey = {k: rolled(ey, k) for k in range(-1, 3)}
            ry1 = {k: rolled(y1, k) for k in range(0, 4)}
            for r in range(4):
                out = jnp.where(seg < 2,
                                jnp.where(seg == 0, ry0[0 - r], ry0[1 - r]),
                                jnp.where(seg == 2, rey[2 - r], ry1[3 - r]))
                kl[gg * 4 + r, pl.ds(r0, 32), :] = pltpu.bitcast(out, i8)

        def q_limbs(ct, o, k):
            r = o * 128 + k * 32
            q = qT[ct, r:r + 32, :].reshape(4, 8, 128)
            a1 = al[ct, o * 8:(o + 1) * 8, :]
            a256 = a1 * 256.0
            x = (q[0] * a1, q[1] * a256, q[2] * a1, q[3] * a256)
            w0, u, x1, w16 = [_pack_rounded(x, e, (cst[2 * i], cst[2 * i + 1]))
                              for i, (e, _) in enumerate(PACKS)]
            for j, word in enumerate((u, w0 - u, x1, w16 - (w0 << 4))):
                r = (4 * j + k) * QS + o * 8
                qw[ct, r:r + 8, :] = word ^ SIGN_BYTES

        def q_raw(r0):
            return jax.lax.dot_general(pltpu.bitcast(wqT[...], bf16), _wide(xns, pl.ds(r0, 128)),
                                       NT, preferred_element_type=f32)

        def qproj(t, bound):
            beta8 = k_stats()
            for cc in range(TA2 // 128):
                ct = t * (TA2 // 128) + cc
                r0 = pl.multiple_of(ct * 128, 128)
                q = q_raw(r0) * tmp[1, 0:D, :]
                qT[ct, 0:D, :] = q
                aq = jnp.abs(q).reshape(4, DH, 8, 128)
                amax = jnp.maximum(jnp.max(aq, axis=1), 1e-30).reshape(H, 128)
                al[ct] = 254.0 / amax
                cs[ct] = amax * (SCALE * LOG2E / (254.0 * 127.0))
                bound = jnp.maximum(bound, jnp.max(jnp.sum(aq, axis=1), axis=0))
                for rb in range(4):
                    for gg in range(4):
                        k_limbs(pl.multiple_of(r0 + rb * 32, 32), gg, beta8)
            return bound
        bound = jax.lax.fori_loop(0, S // TA2, qproj, jnp.zeros((8, 128), f32))

        def vproj(t, _):
            p_c[...] = jnp.zeros(p_c.shape, bf16)
            acc_c[...] = jnp.zeros(acc_c.shape, f32)
            l_c[...] = jnp.ones(l_c.shape, f32)
            v_c[1, S // TK - 1] = jnp.zeros((8, 128), i32)
            for cc in range(TA2 // 128):
                ct = t * (TA2 // 128) + cc
                r0 = pl.multiple_of(ct * 128, 128)
                xn = _wide(xns, pl.ds(r0, 128))
                for o in range(4):
                    rows = slice(o * 128, (o + 1) * 128)
                    wv = pltpu.bitcast(wvT[o * 64:(o + 1) * 64, :], bf16)
                    v = jax.lax.dot_general(wv, xn, NT, preferred_element_type=f32)
                    vT[ct, rows, :] = v.astype(bf16)
                    for k in range(4):
                        q_limbs(ct, o, k)
            return jnp.max(bound)
        bmax = jax.lax.fori_loop(0, S // TA2, vproj, jnp.float32(0))
        safe = (bmax * (SCALE * LOG2E) < SAFE_LOG2) & v_ok

        def o_transpose(t):
            on = oT[:, pl.ds(_aligned(t * TM, TM), TS)].T
            for j in range(ND):
                oN[j] = on[:, j * 128:(j + 1) * 128]

        @pl.when(safe)
        def _fast():
            nq = S // TQ
            nk = S // TK
            cq = TQ // 128

            def head_of(g, b):
                return ((g >> 2) << 3) + 4 * b + (g & 3)

            def pv(v, pb, acc):
                return acc + jnp.dot(pltpu.bitcast(v, bf16), pb, preferred_element_type=f32)

            def finish(h, q0, acc, ls):
                lsum = jnp.sum(ls, axis=0, keepdims=True)
                r = pl.reciprocal(lsum, approx=True)
                r = r * (2.0 - lsum * r)
                oT[pl.ds(_aligned(h * DH, DH), DH), pl.ds(q0, TQ)] = (acc * r).astype(bf16)

            def body(g, _):
                ph, pq0 = head_of(jnp.maximum(g - 1, 0), 1), (nq - 1) * TQ
                pb, acc, pls, pv_last = p_c[...], acc_c[0], l_c[...], v_c[1, nk - 1]
                kg = pltpu.bitcast(kl[g], i32)
                k_c[0] = kg
                k_c[1] = pltpu.roll(kg, 64, 1)
                for b in range(2):
                    h = head_of(g, b)
                    for kc in range(nk):
                        v_c[b, kc] = pltpu.bitcast(
                            vT[kc, pl.ds(_aligned(h * DH, DH), DH), :], i32)
                    for j in range(NC):
                        c_c[b, :, j * 128:(j + 1) * 128] = jnp.broadcast_to(
                            cs[j, pl.ds(h, 1), :], (8, 128))
                zero = jnp.zeros((DH, TQ), i32)
                for qt in range(nq):
                    for b in range(2):
                        h = head_of(g, b)
                        words = jnp.concatenate(
                            [qw[qt * cq + j, pl.ds(h, DH, stride=QS), :] for j in range(cq)],
                            axis=1)
                        w = pltpu.bitcast(jnp.concatenate([words, zero], axis=0), i8)
                        c = c_c[b, :, qt * TQ:(qt + 1) * TQ]
                        ls = None
                        for kc in range(nk):
                            kk = k_c[b, kc * (TK // 4):(kc + 1) * (TK // 4), :]
                            s = jnp.dot(pltpu.bitcast(kk, i8), w, preferred_element_type=i32)
                            if kc == 0:
                                finish(ph, pq0, pv(pv_last, pb, acc), pls)
                                acc = acc_c[1]
                            else:
                                acc = pv(v_c[b, kc - 1], pb, acc)
                            p = jnp.exp2(s.astype(f32).reshape(TK // 8, 8, TQ) * c)
                            psum = jnp.sum(p, axis=0)
                            ls = psum if ls is None else ls + psum
                            pb = p.reshape(TK, TQ).astype(bf16)
                        ph, pq0, pls, pv_last = h, qt * TQ, ls, v_c[b, nk - 1]
                p_c[...] = pb
                acc_c[0] = acc
                l_c[...] = pls
                return 0
            jax.lax.fori_loop(0, NG, body, 0)
            o_transpose(0)
            finish(H - 1, (nq - 1) * TQ, pv(v_c[1, nk - 1], p_c[...], acc_c[0]), l_c[...])

        @pl.when(jnp.logical_not(safe))
        def _slow():
            def qraw(ct, _):
                qT[ct, 0:D, :] = q_raw(pl.multiple_of(ct * 128, 128))
                return 0
            jax.lax.fori_loop(0, NC, qraw, 0)

            def body(i, _):
                h = i // NC
                ct = i % NC
                q0 = pl.multiple_of(ct * 128, 128)
                g0 = pl.multiple_of((h // 8) * 128, 128)
                r0 = pl.multiple_of(h * DH, DH)
                qh = qT[ct, pl.ds(g0 + h % 8, DH, stride=8), :]
                row = jax.lax.broadcasted_iota(i32, (128, 128), 0)
                w = jnp.where(row // DH == h % 8, jnp.concatenate([qh] * 8, axis=0), 0.0)
                kb = kf[:, pl.ds(g0, 128)].astype(bf16)
                s = jnp.dot(kb, w.astype(bf16), preferred_element_type=f32) * SCALE
                m = jnp.max(s, axis=0, keepdims=True)
                p = jnp.exp(s - m)
                lsum = jnp.sum(p, axis=0, keepdims=True)
                acc = jnp.dot(_wide(vT, pl.ds(r0, DH)), p.astype(bf16),
                              preferred_element_type=f32)
                oT[pl.ds(r0, DH), pl.ds(q0, 128)] = (acc / lsum).astype(bf16)
                return 0
            jax.lax.fori_loop(0, H * NC, body, 0)
            o_transpose(0)

        def ffn(t, last):
            ns = TM // TS
            rs = [pl.multiple_of(t * TM + u * TS, TS) for u in range(ns)]
            b1 = b1f[...]
            b2 = b2f[...]
            x0 = [(xs if last else xb)[pl.ds(r, TS), :].astype(f32) for r in rs]
            x1 = [x0[0] + jnp.dot(_wide(oN), wo[...], preferred_element_type=f32)]
            x1 += [x + jax.lax.dot_general(
                oT[:, pl.ds(r, TS)], wo[...], TN, preferred_element_type=f32)
                for r, x in zip(rs[1:], x0[1:])]
            o_transpose(jnp.minimum(t + 1, S // TM - 1))
            hh = [_gelu(jnp.dot(_layernorm(x).astype(bf16), w1[...],
                                preferred_element_type=f32) + b1).astype(bf16) for x in x1]
            x2 = []
            for u, (r, x, g) in enumerate(zip(rs, x1, hh)):
                x = x + jnp.dot(g, w2[...], preferred_element_type=f32) + b2
                if last:
                    xb[pl.ds(r, TS), :] = x.astype(bf16)
                    out_copy(t * ns + u).start()
                else:
                    xs[pl.ds(r, TS), :] = x
                    x2.append(x)
            if not last:
                km = kmx[...]
                for r, x in zip(rs, x2):
                    km = jnp.maximum(km, k_proj(ln_store(x, r, TS), r, TS))
                kmx[...] = km
            return 0

        @pl.when(li == 0)
        def _():
            for cp in late:
                cp.wait()
            b1f[...] = b1v[...].astype(f32).reshape(1, F)
            b2f[...] = b2v[...].astype(f32).reshape(1, D)

        @pl.when(li < N_LAYERS - 1)
        def _():
            kmx[...] = jnp.zeros(kmx.shape, f32)
            jax.lax.fori_loop(0, S // TM, lambda t, _: ffn(t, False), 0)

        @pl.when(li == N_LAYERS - 1)
        def _():
            jax.lax.fori_loop(0, S // TM, lambda t, _: ffn(t, True), 0)
        return carry

    jax.lax.fori_loop(0, N_LAYERS, layer, 0)
    for u in range(S // TS):
        out_copy(u).wait()


@jax.jit
def pallas_interleave_layers__mha_block__dense_activation_gelu__prompt_kernel(
    A_x: jax.Array,
    A_wqkv: jax.Array,
    A_wo: jax.Array,
    B_x: jax.Array,
    B_w1: jax.Array,
    B_b1: jax.Array,
    B_w2: jax.Array,
    B_b2: jax.Array,
):
    del B_x
    hbm = pl.BlockSpec(memory_space=pl.ANY)
    out = pl.pallas_call(
        _kernel,
        out_shape=jax.ShapeDtypeStruct((S, D), A_x.dtype),
        in_specs=[hbm] * 7,
        out_specs=hbm,
        scratch_shapes=[
            pltpu.VMEM((S, D), bf16),
            pltpu.VMEM((3, D, D), bf16),
            pltpu.VMEM((D, D), bf16),
            pltpu.VMEM((D, F), bf16),
            pltpu.VMEM((F, D), bf16),
            pltpu.SemaphoreType.DMA((NX + 8 + S // TS,)),
            pltpu.VMEM((S, D), f32),
            pltpu.VMEM((ND, S, 128), bf16),
            pltpu.VMEM((D // 2, D), i32),
            pltpu.VMEM((D // 2, D), i32),
            pltpu.VMEM((ND, (H + 1) * HS, 128), f32),
            pltpu.VMEM((S, D), f32),
            pltpu.VMEM((8, D), f32),
            pltpu.VMEM((NC, D + 8, 128), f32),
            pltpu.VMEM((NC, D, 128), bf16),
            pltpu.VMEM((NG, S, 128), i8),
            pltpu.VMEM((NC, (DH + 1) * QS, 128), i32),
            pltpu.VMEM((NC, H, 128), f32),
            pltpu.VMEM((NC, H, 128), f32),
            pltpu.VMEM((D, S), bf16),
            pltpu.VMEM((ND, TS, 128), bf16),
            pltpu.VMEM((TK, TQ), bf16),
            pltpu.VMEM((2, DH, TQ), f32),
            pltpu.VMEM((8, TQ), f32),
            pltpu.VMEM((2, S // 4, 128), i32),
            pltpu.VMEM((2, NC, 8, 128), i32),
            pltpu.VMEM((2, 8, S), f32),
            pltpu.VMEM((8, 8, 128), f32),
            pltpu.VMEM((F,), bf16),
            pltpu.VMEM((D,), bf16),
            pltpu.VMEM((1, F), f32),
            pltpu.VMEM((1, D), f32),
        ],
        compiler_params=pltpu.CompilerParams(vmem_limit_bytes=100 * 1024 * 1024),
    )(A_x.reshape(S, D), A_wqkv, A_wo, B_w1, B_b1, B_w2, B_b2)
    return out.reshape(1, S, D)
```

```python
import jax
import jax.numpy as jnp
import jax.experimental.pallas as pl
import jax.experimental.pallas.tpu as pltpu

S, D, H, DH, F = 2048, 512, 32, 16, 1792
N_LAYERS = 2
EPS = 1e-5
LOG2E = 1.4426950408889634
SCALE = DH ** -0.5
MAGIC = 12582912.0

SIGN_BYTES = 0x80808080 - 2 ** 32

NG = H // 2
NC = S // 128
ND = D // 128
X_CHUNKS = ((0, 256), (256, 256), (512, 768), (1280, 768))
NX = len(X_CHUNKS)
TA = 256
W_AT = 4
TA2 = 1024
TM = 512
TS = 128
TQ = 1024
TK = 128
HS = 24
QS = 40

SAFE_LOG2 = 64.0
WV_MIN, WV_MAX = 2.0 ** -20, 2.0 ** 20

bf16 = jnp.bfloat16
f32 = jnp.float32
i32 = jnp.int32
i8 = jnp.int8
NT = (((1,), (1,)), ((), ()))
TN = (((0,), (0,)), ((), ()))


def _layernorm(x):
    m = jnp.mean(x, axis=-1, keepdims=True)
    xc = x - m
    v = jnp.mean(xc * xc, axis=-1, keepdims=True)
    return xc * jax.lax.rsqrt(v + EPS)


def _gelu(x):
    c = 0.7978845608028654
    return 0.5 * x * (1.0 + jnp.tanh(c * (x + 0.044715 * (x * x * x))))


def _bits(t):
    return pltpu.bitcast(t, i32)


PACKS = ((0, 256), (1, 128), (4, 128), (-4, 16 * 256 + 128))
BIG = 2.0 ** 31 + 2.0 ** 21


def _pack_consts(e, off):
    return [(BIG - 2.0 ** 23 - 257 * off - extra) * 2.0 ** e
            for extra in (0, 2 ** 16 - ((150 + e) << 7))]


def _pack_rounded(x, e, sub):
    def pair(lo, hi256, c):
        return _bits(((hi256 + BIG * 2.0 ** e) - c) + lo)
    return pair(x[0], x[1], sub[0]) + (pair(x[2], x[3], sub[1]) << 16)


def _wide(ref, rows=slice(None)):
    return jnp.concatenate([ref[j, rows, :] for j in range(ref.shape[0])], axis=1)


def _aligned(i, n):
    return i if isinstance(i, int) else pl.multiple_of(i, n)


def _kernel(x_hbm, wqkv_hbm, wo_hbm, w1_hbm, b1_hbm, w2_hbm, b2_hbm, o_hbm,
            xb, wqkv, wo, w1, w2, sems,
            xs, xns, wqT, wvT, tmp, kf, kmx, qT, vT, kl, qw, cs, al, oT, oN,
            p_c, acc_c, l_c, k_c, v_c, c_c, cst, b1v, b2v, b1f, b2f):

    def x_copy(c):
        r0, n = X_CHUNKS[c]
        return pltpu.make_async_copy(x_hbm.at[pl.ds(r0, n), :], xb.at[pl.ds(r0, n), :],
                                     sems.at[c])

    def wqkv_copy(j):
        return pltpu.make_async_copy(wqkv_hbm.at[:, pl.ds(j * D, D)], wqkv.at[j],
                                     sems.at[NX + j])

    late = [pltpu.make_async_copy(src, dst, sems.at[NX + 3]) for src, dst in
            ((wo_hbm, wo), (w1_hbm, w1), (w2_hbm, w2), (b1_hbm, b1v), (b2_hbm, b2v))]

    def out_copy(u):
        r0 = _aligned(u * TS, TS)
        return pltpu.make_async_copy(xb.at[pl.ds(r0, TS), :], o_hbm.at[pl.ds(r0, TS), :],
                                     sems.at[NX + 4])

    x_copy(0).start()
    wqkv_copy(1).start()
    for c in range(1, NX):
        x_copy(c).start()
    wqkv_copy(0).start()
    wqkv_copy(2).start()
    for cp in late:
        cp.start()

    for i, (e, off) in enumerate(PACKS):
        for j, c in enumerate(_pack_consts(e, off)):
            cst[2 * i + j] = jnp.full((8, 128), c, f32)

    for ct in range(NC):
        for j in range(DH):
            qw[ct, j * QS + H:(j + 1) * QS, :] = jnp.zeros((QS - H, 128), i32)
        qw[ct, DH * QS:, :] = jnp.zeros((QS, 128), i32)
        qT[ct, D:, :] = jnp.zeros((8, 128), f32)
    for j in range(ND):
        for h in range(H):
            tmp[j, h * HS + DH:(h + 1) * HS, :] = jnp.zeros((HS - DH, 128), f32)
        tmp[j, H * HS:, :] = jnp.zeros((HS, 128), f32)

    def ln_store(x, r0, n):
        xn = _layernorm(x).astype(bf16)
        for j in range(ND):
            xns[j, pl.ds(r0, n), :] = xn[:, j * 128:(j + 1) * 128]
        return xn

    def k_proj(xn, r0, n):
        k = jnp.dot(xn, wqkv[1], preferred_element_type=f32)
        kf[pl.ds(r0, n), :] = k
        return jnp.max(jnp.abs(k).reshape(n // 8, 8, D), axis=0)

    def first_ln(u):
        ln_store(xb[u * TA:(u + 1) * TA, :].astype(f32), u * TA, TA)

    def w_transposes(j):
        cols = slice(j * 128, (j + 1) * 128)
        wv = wqkv[2, cols, :]
        wvT[:, cols] = pltpu.bitcast(wv.T, i32)
        wq_t = wqkv[0, cols, :].T.astype(f32)
        for h in range(H):
            tmp[j, h * HS:h * HS + DH, :] = wq_t[h * DH:(h + 1) * DH]
        for o in range(4):
            for d2 in range(DH // 2):
                r = o * 64 + d2 * 8
                wqT[r:r + 8, cols] = pltpu.bitcast(jnp.concatenate(
                    [tmp[j, pl.ds(o * 8 * HS + 2 * d2 + e, 8, stride=HS), :]
                     for e in range(2)], axis=0).astype(bf16), i32)
        return jnp.max(jnp.abs(wv.astype(f32)).reshape(16, 8, D), axis=0)

    x_copy(0).wait()
    first_ln(0)
    kmax8 = jnp.zeros((8, D), f32)
    wv_max = jnp.zeros((8, D), f32)
    starts = {r0 // TA: c for c, (r0, _) in enumerate(X_CHUNKS)}
    for u in range(S // TA):
        if u == 0:
            wqkv_copy(1).wait()
        if u + 1 in starts:
            x_copy(starts[u + 1]).wait()
        if u == W_AT:
            wqkv_copy(0).wait()
            wqkv_copy(2).wait()
        if u >= W_AT:
            wv_max = jnp.maximum(wv_max, w_transposes(u - W_AT))
        kmax8 = jnp.maximum(kmax8, k_proj(_wide(xns, slice(u * TA, (u + 1) * TA)), u * TA, TA))
        if u + 1 < S // TA:
            first_ln(u + 1)
    kmx[...] = kmax8
    wv_max = jnp.max(wv_max)
    v_ok = (wv_max >= WV_MIN) & (wv_max <= WV_MAX)

    def layer(li, carry):
        def k_stats():
            kmax = jnp.maximum(jnp.max(kmx[...], axis=0, keepdims=True), 1e-30)
            kc = jnp.broadcast_to(kmax, (128, D)).T
            for h in range(H):
                tmp[0, h * HS:h * HS + DH, :] = kc[h * DH:(h + 1) * DH]
            for o in range(4):
                for d in range(DH):
                    r = o * 128 + d * 8
                    tmp[1, r:r + 8, :] = tmp[0, pl.ds(o * 8 * HS + d, 8, stride=HS), :]
            return jnp.broadcast_to(127.0 / kmax, (8, D))

        def k_limbs(r0, gg, beta8):
            seg = (jax.lax.broadcasted_iota(i32, (8, 128), 1) // DH) % 4
            y = kf[pl.ds(r0, 32), gg * 128:(gg + 1) * 128].reshape(4, 8, 128) \
                * beta8[:, gg * 128:(gg + 1) * 128]
            t0 = _bits(y + MAGIC)
            te = _bits(y + MAGIC / 16) - (t0 << 4)
            t1 = _bits(y + MAGIC * 16)
            y0, ey, y1 = [pltpu.bitcast(a.reshape(32, 128).astype(i8), i32)
                          for a in (t0, te, t1)]

            def rolled(a, k):
                return a if k == 0 else pltpu.roll(a, (DH * k) % 128, 1)
            ry0 = {k: rolled(y0, k) for k in range(-3, 2)}
            rey = {k: rolled(ey, k) for k in range(-1, 3)}
            ry1 = {k: rolled(y1, k) for k in range(0, 4)}
            for r in range(4):
                out = jnp.where(seg < 2,
                                jnp.where(seg == 0, ry0[0 - r], ry0[1 - r]),
                                jnp.where(seg == 2, rey[2 - r], ry1[3 - r]))
                kl[gg * 4 + r, pl.ds(r0, 32), :] = pltpu.bitcast(out, i8)

        def q_limbs(ct, o, k):
            r = o * 128 + k * 32
            q = qT[ct, r:r + 32, :].reshape(4, 8, 128)
            a1 = al[ct, o * 8:(o + 1) * 8, :]
            a256 = a1 * 256.0
            x = (q[0] * a1, q[1] * a256, q[2] * a1, q[3] * a256)
            w0, u, x1, w16 = [_pack_rounded(x, e, (cst[2 * i], cst[2 * i + 1]))
                              for i, (e, _) in enumerate(PACKS)]
            for j, word in enumerate((u, w0 - u, x1, w16 - (w0 << 4))):
                r = (4 * j + k) * QS + o * 8
                qw[ct, r:r + 8, :] = word ^ SIGN_BYTES

        def q_raw(r0):
            return jax.lax.dot_general(pltpu.bitcast(wqT[...], bf16), _wide(xns, pl.ds(r0, 128)),
                                       NT, preferred_element_type=f32)

        def qproj(t, bound):
            beta8 = k_stats()
            for cc in range(TA2 // 128):
                ct = t * (TA2 // 128) + cc
                r0 = pl.multiple_of(ct * 128, 128)
                q = q_raw(r0) * tmp[1, 0:D, :]
                qT[ct, 0:D, :] = q
                aq = jnp.abs(q).reshape(4, DH, 8, 128)
                amax = jnp.maximum(jnp.max(aq, axis=1), 1e-30).reshape(H, 128)
                al[ct] = 254.0 / amax
                cs[ct] = amax * (SCALE * LOG2E / (254.0 * 127.0))
                bound = jnp.maximum(bound, jnp.max(jnp.sum(aq, axis=1), axis=0))
                for rb in range(4):
                    for gg in range(4):
                        k_limbs(pl.multiple_of(r0 + rb * 32, 32), gg, beta8)
            return bound
        bound = jax.lax.fori_loop(0, S // TA2, qproj, jnp.zeros((8, 128), f32))

        def vproj(t, _):
            p_c[...] = jnp.zeros(p_c.shape, bf16)
            acc_c[...] = jnp.zeros(acc_c.shape, f32)
            l_c[...] = jnp.ones(l_c.shape, f32)
            v_c[1, S // TK - 1] = jnp.zeros((8, 128), i32)
            for cc in range(TA2 // 128):
                ct = t * (TA2 // 128) + cc
                r0 = pl.multiple_of(ct * 128, 128)
                xn = _wide(xns, pl.ds(r0, 128))
                for o in range(4):
                    rows = slice(o * 128, (o + 1) * 128)
                    wv = pltpu.bitcast(wvT[o * 64:(o + 1) * 64, :], bf16)
                    v = jax.lax.dot_general(wv, xn, NT, preferred_element_type=f32)
                    vT[ct, rows, :] = v.astype(bf16)
                    for k in range(4):
                        q_limbs(ct, o, k)
            return jnp.max(bound)
        bmax = jax.lax.fori_loop(0, S // TA2, vproj, jnp.float32(0))
        safe = (bmax * (SCALE * LOG2E) < SAFE_LOG2) & v_ok

        def o_transpose(t):
            on = oT[:, pl.ds(_aligned(t * TM, TM), TS)].T
            for j in range(ND):
                oN[j] = on[:, j * 128:(j + 1) * 128]

        @pl.when(safe)
        def _fast():
            nq = S // TQ
            nk = S // TK
            cq = TQ // 128

            def head_of(g, b):
                return ((g >> 2) << 3) + 4 * b + (g & 3)

            def pv(v, pb, acc):
                return acc + jnp.dot(pltpu.bitcast(v, bf16), pb, preferred_element_type=f32)

            def finish(h, q0, acc, ls):
                lsum = jnp.sum(ls, axis=0, keepdims=True)
                r = pl.reciprocal(lsum, approx=True)
                r = r * (2.0 - lsum * r)
                oT[pl.ds(_aligned(h * DH, DH), DH), pl.ds(q0, TQ)] = (acc * r).astype(bf16)

            def body(g, _):
                ph, pq0 = head_of(jnp.maximum(g - 1, 0), 1), (nq - 1) * TQ
                pb, acc, pls, pv_last = p_c[...], acc_c[0], l_c[...], v_c[1, nk - 1]
                kg = pltpu.bitcast(kl[g], i32)
                k_c[0] = kg
                k_c[1] = pltpu.roll(kg, 64, 1)
                for b in range(2):
                    h = head_of(g, b)
                    for kc in range(nk):
                        v_c[b, kc] = pltpu.bitcast(
                            vT[kc, pl.ds(_aligned(h * DH, DH), DH), :], i32)
                    for j in range(NC):
                        c_c[b, :, j * 128:(j + 1) * 128] = jnp.broadcast_to(
                            cs[j, pl.ds(h, 1), :], (8, 128))
                zero = jnp.zeros((DH, TQ), i32)
                for qt in range(nq):
                    for b in range(2):
                        h = head_of(g, b)
                        words = jnp.concatenate(
                            [qw[qt * cq + j, pl.ds(h, DH, stride=QS), :] for j in range(cq)],
                            axis=1)
                        w = pltpu.bitcast(jnp.concatenate([words, zero], axis=0), i8)
                        c = c_c[b, :, qt * TQ:(qt + 1) * TQ]
                        ls = None
                        for kc in range(nk):
                            kk = k_c[b, kc * (TK // 4):(kc + 1) * (TK // 4), :]
                            s = jnp.dot(pltpu.bitcast(kk, i8), w, preferred_element_type=i32)
                            if kc == 0:
                                finish(ph, pq0, pv(pv_last, pb, acc), pls)
                                acc = acc_c[1]
                            else:
                                acc = pv(v_c[b, kc - 1], pb, acc)
                            p = jnp.exp2(s.astype(f32).reshape(TK // 8, 8, TQ) * c)
                            psum = jnp.sum(p, axis=0)
                            ls = psum if ls is None else ls + psum
                            pb = p.reshape(TK, TQ).astype(bf16)
                        ph, pq0, pls, pv_last = h, qt * TQ, ls, v_c[b, nk - 1]
                p_c[...] = pb
                acc_c[0] = acc
                l_c[...] = pls
                return 0
            jax.lax.fori_loop(0, NG, body, 0)
            o_transpose(0)
            finish(H - 1, (nq - 1) * TQ, pv(v_c[1, nk - 1], p_c[...], acc_c[0]), l_c[...])

        @pl.when(jnp.logical_not(safe))
        def _slow():
            def qraw(ct, _):
                qT[ct, 0:D, :] = q_raw(pl.multiple_of(ct * 128, 128))
                return 0
            jax.lax.fori_loop(0, NC, qraw, 0)

            def body(i, _):
                h = i // NC
                ct = i % NC
                q0 = pl.multiple_of(ct * 128, 128)
                g0 = pl.multiple_of((h // 8) * 128, 128)
                r0 = pl.multiple_of(h * DH, DH)
                qh = qT[ct, pl.ds(g0 + h % 8, DH, stride=8), :]
                row = jax.lax.broadcasted_iota(i32, (128, 128), 0)
                w = jnp.where(row // DH == h % 8, jnp.concatenate([qh] * 8, axis=0), 0.0)
                kb = kf[:, pl.ds(g0, 128)].astype(bf16)
                s = jnp.dot(kb, w.astype(bf16), preferred_element_type=f32) * SCALE
                m = jnp.max(s, axis=0, keepdims=True)
                p = jnp.exp(s - m)
                lsum = jnp.sum(p, axis=0, keepdims=True)
                acc = jnp.dot(_wide(vT, pl.ds(r0, DH)), p.astype(bf16),
                              preferred_element_type=f32)
                oT[pl.ds(r0, DH), pl.ds(q0, 128)] = (acc / lsum).astype(bf16)
                return 0
            jax.lax.fori_loop(0, H * NC, body, 0)
            o_transpose(0)

        def ffn(t, last):
            ns = TM // TS
            rs = [pl.multiple_of(t * TM + u * TS, TS) for u in range(ns)]
            b1 = b1f[...]
            b2 = b2f[...]
            x0 = [(xs if last else xb)[pl.ds(r, TS), :].astype(f32) for r in rs]
            x1 = [x0[0] + jnp.dot(_wide(oN), wo[...], preferred_element_type=f32)]
            x1 += [x + jax.lax.dot_general(
                oT[:, pl.ds(r, TS)], wo[...], TN, preferred_element_type=f32)
                for r, x in zip(rs[1:], x0[1:])]
            o_transpose(jnp.minimum(t + 1, S // TM - 1))
            hh = [_gelu(jnp.dot(_layernorm(x).astype(bf16), w1[...],
                                preferred_element_type=f32) + b1).astype(bf16) for x in x1]
            x2 = []
            for u, (r, x, g) in enumerate(zip(rs, x1, hh)):
                x = x + jnp.dot(g, w2[...], preferred_element_type=f32) + b2
                if last:
                    xb[pl.ds(r, TS), :] = x.astype(bf16)
                    out_copy(t * ns + u).start()
                else:
                    xs[pl.ds(r, TS), :] = x
                    x2.append(x)
            if not last:
                km = kmx[...]
                for r, x in zip(rs, x2):
                    km = jnp.maximum(km, k_proj(ln_store(x, r, TS), r, TS))
                kmx[...] = km
            return 0

        @pl.when(li == 0)
        def _():
            for cp in late:
                cp.wait()
            b1f[...] = b1v[...].astype(f32).reshape(1, F)
            b2f[...] = b2v[...].astype(f32).reshape(1, D)

        @pl.when(li < N_LAYERS - 1)
        def _():
            kmx[...] = jnp.zeros(kmx.shape, f32)
            jax.lax.fori_loop(0, S // TM, lambda t, _: ffn(t, False), 0)

        @pl.when(li == N_LAYERS - 1)
        def _():
            jax.lax.fori_loop(0, S // TM, lambda t, _: ffn(t, True), 0)
        return carry

    jax.lax.fori_loop(0, N_LAYERS, layer, 0)
    for u in range(S // TS):
        out_copy(u).wait()


@jax.jit
def pallas_interleave_layers__mha_block__dense_activation_gelu__prompt_kernel(
    A_x: jax.Array,
    A_wqkv: jax.Array,
    A_wo: jax.Array,
    B_x: jax.Array,
    B_w1: jax.Array,
    B_b1: jax.Array,
    B_w2: jax.Array,
    B_b2: jax.Array,
):
    del B_x
    hbm = pl.BlockSpec(memory_space=pl.ANY)
    out = pl.pallas_call(
        _kernel,
        out_shape=jax.ShapeDtypeStruct((S, D), A_x.dtype),
        in_specs=[hbm] * 7,
        out_specs=hbm,
        scratch_shapes=[
            pltpu.VMEM((S, D), bf16),
            pltpu.VMEM((3, D, D), bf16),
            pltpu.VMEM((D, D), bf16),
            pltpu.VMEM((D, F), bf16),
            pltpu.VMEM((F, D), bf16),
            pltpu.SemaphoreType.DMA((NX + 5,)),
            pltpu.VMEM((S, D), f32),
            pltpu.VMEM((ND, S, 128), bf16),
            pltpu.VMEM((D // 2, D), i32),
            pltpu.VMEM((D // 2, D), i32),
            pltpu.VMEM((ND, (H + 1) * HS, 128), f32),
            pltpu.VMEM((S, D), f32),
            pltpu.VMEM((8, D), f32),
            pltpu.VMEM((NC, D + 8, 128), f32),
            pltpu.VMEM((NC, D, 128), bf16),
            pltpu.VMEM((NG, S, 128), i8),
            pltpu.VMEM((NC, (DH + 1) * QS, 128), i32),
            pltpu.VMEM((NC, H, 128), f32),
            pltpu.VMEM((NC, H, 128), f32),
            pltpu.VMEM((D, S), bf16),
            pltpu.VMEM((ND, TS, 128), bf16),
            pltpu.VMEM((TK, TQ), bf16),
            pltpu.VMEM((2, DH, TQ), f32),
            pltpu.VMEM((8, TQ), f32),
            pltpu.VMEM((2, S // 4, 128), i32),
            pltpu.VMEM((2, NC, 8, 128), i32),
            pltpu.VMEM((2, 8, S), f32),
            pltpu.VMEM((8, 8, 128), f32),
            pltpu.VMEM((F,), bf16),
            pltpu.VMEM((D,), bf16),
            pltpu.VMEM((1, F), f32),
            pltpu.VMEM((1, D), f32),
        ],
        compiler_params=pltpu.CompilerParams(vmem_limit_bytes=100 * 1024 * 1024),
    )(A_x.reshape(S, D), A_wqkv, A_wo, B_w1, B_b1, B_w2, B_b2)
    return out.reshape(1, S, D)
```

```python
import jax
import jax.numpy as jnp
import jax.experimental.pallas as pl
import jax.experimental.pallas.tpu as pltpu

S, D, H, DH, F = 2048, 512, 32, 16, 1792
N_LAYERS = 2
EPS = 1e-5
LOG2E = 1.4426950408889634
SCALE = DH ** -0.5
MAGIC = 12582912.0

SIGN_BYTES = 0x80808080 - 2 ** 32

NG = H // 2
NC = S // 128
ND = D // 128
X_CHUNKS = ((0, 256), (256, 256), (512, 768), (1280, 768))
NX = len(X_CHUNKS)
TA = 256
W_AT = 4
TA2 = 1024
TM = 512
TS = 128
TQ = 1024
TK = 128
HS = 24
QS = 40

SAFE_LOG2 = 64.0
WV_MIN, WV_MAX = 2.0 ** -20, 2.0 ** 20

bf16 = jnp.bfloat16
f32 = jnp.float32
i32 = jnp.int32
i8 = jnp.int8
NT = (((1,), (1,)), ((), ()))
TN = (((0,), (0,)), ((), ()))


def _layernorm(x):
    m = jnp.mean(x, axis=-1, keepdims=True)
    xc = x - m
    v = jnp.mean(xc * xc, axis=-1, keepdims=True)
    return xc * jax.lax.rsqrt(v + EPS)


def _gelu(x):
    c = 0.7978845608028654
    return 0.5 * x * (1.0 + jnp.tanh(c * (x + 0.044715 * (x * x * x))))


def _bits(t):
    return pltpu.bitcast(t, i32)


PACKS = ((0, 256), (1, 128), (4, 128), (-4, 16 * 256 + 128))
BIG = 2.0 ** 31 + 2.0 ** 21


def _pack_consts(e, off):
    return [(BIG - 2.0 ** 23 - 257 * off - extra) * 2.0 ** e
            for extra in (0, 2 ** 16 - ((150 + e) << 7))]


def _pack_rounded(x, e, sub):
    def pair(lo, hi256, c):
        return _bits(((hi256 + BIG * 2.0 ** e) - c) + lo)
    return pair(x[0], x[1], sub[0]) + (pair(x[2], x[3], sub[1]) << 16)


def _wide(ref, rows=slice(None)):
    return jnp.concatenate([ref[j, rows, :] for j in range(ref.shape[0])], axis=1)


def _aligned(i, n):
    return i if isinstance(i, int) else pl.multiple_of(i, n)


def _kernel(x_hbm, wqkv_hbm, wo_hbm, w1_hbm, b1_hbm, w2_hbm, b2_hbm, o_hbm,
            xb, wqkv, wo, w1, w2, sems,
            xs, xns, wqT, wvT, tmp, kf, kmx, qT, vT, kl, qw, cs, al, oT, oN,
            p_c, acc_c, l_c, k_c, v_c, c_c, cst, b1v, b2v, b1f, b2f):

    def x_copy(c):
        r0, n = X_CHUNKS[c]
        return pltpu.make_async_copy(x_hbm.at[pl.ds(r0, n), :], xb.at[pl.ds(r0, n), :],
                                     sems.at[c])

    def wqkv_copy(j):
        return pltpu.make_async_copy(wqkv_hbm.at[:, pl.ds(j * D, D)], wqkv.at[j],
                                     sems.at[NX + j])

    late = [pltpu.make_async_copy(src, dst, sems.at[NX + 3]) for src, dst in
            ((wo_hbm, wo), (w1_hbm, w1), (w2_hbm, w2), (b1_hbm, b1v), (b2_hbm, b2v))]

    def out_copy(u):
        r0 = _aligned(u * TS, TS)
        return pltpu.make_async_copy(xb.at[pl.ds(r0, TS), :], o_hbm.at[pl.ds(r0, TS), :],
                                     sems.at[NX + 4])

    x_copy(0).start()
    wqkv_copy(1).start()
    for c in range(1, NX):
        x_copy(c).start()
    wqkv_copy(0).start()
    wqkv_copy(2).start()
    for cp in late:
        cp.start()

    for i, (e, off) in enumerate(PACKS):
        for j, c in enumerate(_pack_consts(e, off)):
            cst[2 * i + j] = jnp.full((8, 128), c, f32)

    for ct in range(NC):
        for j in range(DH):
            qw[ct, j * QS + H:(j + 1) * QS, :] = jnp.zeros((QS - H, 128), i32)
        qw[ct, DH * QS:, :] = jnp.zeros((QS, 128), i32)
        qT[ct, D:, :] = jnp.zeros((8, 128), f32)
    for j in range(ND):
        for h in range(H):
            tmp[j, h * HS + DH:(h + 1) * HS, :] = jnp.zeros((HS - DH, 128), f32)
        tmp[j, H * HS:, :] = jnp.zeros((HS, 128), f32)

    def ln_store(x, r0, n):
        xn = _layernorm(x).astype(bf16)
        for j in range(ND):
            xns[j, pl.ds(r0, n), :] = xn[:, j * 128:(j + 1) * 128]
        return xn

    def k_proj(xn, r0, n):
        k = jnp.dot(xn, wqkv[1], preferred_element_type=f32)
        kf[pl.ds(r0, n), :] = k
        return jnp.max(jnp.abs(k).reshape(n // 8, 8, D), axis=0)

    def first_ln(u):
        ln_store(xb[u * TA:(u + 1) * TA, :].astype(f32), u * TA, TA)

    def w_transposes(j):
        cols = slice(j * 128, (j + 1) * 128)
        wv = wqkv[2, cols, :]
        wvT[:, cols] = pltpu.bitcast(wv.T, i32)
        wq_t = wqkv[0, cols, :].T.astype(f32)
        for h in range(H):
            tmp[j, h * HS:h * HS + DH, :] = wq_t[h * DH:(h + 1) * DH]
        for o in range(4):
            for d2 in range(DH // 2):
                r = o * 64 + d2 * 8
                wqT[r:r + 8, cols] = pltpu.bitcast(jnp.concatenate(
                    [tmp[j, pl.ds(o * 8 * HS + 2 * d2 + e, 8, stride=HS), :]
                     for e in range(2)], axis=0).astype(bf16), i32)
        return jnp.max(jnp.abs(wv.astype(f32)).reshape(16, 8, D), axis=0)

    x_copy(0).wait()
    first_ln(0)
    kmax8 = jnp.zeros((8, D), f32)
    wv_max = jnp.zeros((8, D), f32)
    starts = {r0 // TA: c for c, (r0, _) in enumerate(X_CHUNKS)}
    for u in range(S // TA):
        if u == 0:
            wqkv_copy(1).wait()
        if u + 1 in starts:
            x_copy(starts[u + 1]).wait()
        if u == W_AT:
            wqkv_copy(0).wait()
            wqkv_copy(2).wait()
        if u >= W_AT:
            wv_max = jnp.maximum(wv_max, w_transposes(u - W_AT))
        kmax8 = jnp.maximum(kmax8, k_proj(_wide(xns, slice(u * TA, (u + 1) * TA)), u * TA, TA))
        if u + 1 < S // TA:
            first_ln(u + 1)
    kmx[...] = kmax8
    wv_max = jnp.max(wv_max)
    v_ok = (wv_max >= WV_MIN) & (wv_max <= WV_MAX)

    def layer(li, carry):
        def k_stats():
            kmax = jnp.maximum(jnp.max(kmx[...], axis=0, keepdims=True), 1e-30)
            kc = jnp.broadcast_to(kmax, (128, D)).T
            for h in range(H):
                tmp[0, h * HS:h * HS + DH, :] = kc[h * DH:(h + 1) * DH]
            for o in range(4):
                for d in range(DH):
                    r = o * 128 + d * 8
                    tmp[1, r:r + 8, :] = tmp[0, pl.ds(o * 8 * HS + d, 8, stride=HS), :]
            return jnp.broadcast_to(127.0 / kmax, (8, D))

        def k_limbs(r0, gg, beta8):
            seg = (jax.lax.broadcasted_iota(i32, (8, 128), 1) // DH) % 4
            y = kf[pl.ds(r0, 32), gg * 128:(gg + 1) * 128].reshape(4, 8, 128) \
                * beta8[:, gg * 128:(gg + 1) * 128]
            t0 = _bits(y + MAGIC)
            te = _bits(y + MAGIC / 16) - (t0 << 4)
            t1 = _bits(y + MAGIC * 16)
            y0, ey, y1 = [pltpu.bitcast(a.reshape(32, 128).astype(i8), i32)
                          for a in (t0, te, t1)]

            def rolled(a, k):
                return a if k == 0 else pltpu.roll(a, (DH * k) % 128, 1)
            ry0 = {k: rolled(y0, k) for k in range(-3, 2)}
            rey = {k: rolled(ey, k) for k in range(-1, 3)}
            ry1 = {k: rolled(y1, k) for k in range(0, 4)}
            for r in range(4):
                out = jnp.where(seg < 2,
                                jnp.where(seg == 0, ry0[0 - r], ry0[1 - r]),
                                jnp.where(seg == 2, rey[2 - r], ry1[3 - r]))
                kl[gg * 4 + r, pl.ds(r0, 32), :] = pltpu.bitcast(out, i8)

        def q_limbs(ct, o, k):
            r = o * 128 + k * 32
            q = qT[ct, r:r + 32, :].reshape(4, 8, 128)
            a1 = al[ct, o * 8:(o + 1) * 8, :]
            a256 = a1 * 256.0
            x = (q[0] * a1, q[1] * a256, q[2] * a1, q[3] * a256)
            w0, u, x1, w16 = [_pack_rounded(x, e, (cst[2 * i], cst[2 * i + 1]))
                              for i, (e, _) in enumerate(PACKS)]
            for j, word in enumerate((u, w0 - u, x1, w16 - (w0 << 4))):
                r = (4 * j + k) * QS + o * 8
                qw[ct, r:r + 8, :] = word ^ SIGN_BYTES

        def q_raw(r0):
            return jax.lax.dot_general(pltpu.bitcast(wqT[...], bf16), _wide(xns, pl.ds(r0, 128)),
                                       NT, preferred_element_type=f32)

        def qproj(t, bound):
            beta8 = k_stats()
            for cc in range(TA2 // 128):
                ct = t * (TA2 // 128) + cc
                r0 = pl.multiple_of(ct * 128, 128)
                q = q_raw(r0) * tmp[1, 0:D, :]
                qT[ct, 0:D, :] = q
                aq = jnp.abs(q).reshape(4, DH, 8, 128)
                amax = jnp.maximum(jnp.max(aq, axis=1), 1e-30).reshape(H, 128)
                al[ct] = 254.0 / amax
                cs[ct] = amax * (SCALE * LOG2E / (254.0 * 127.0))
                bound = jnp.maximum(bound, jnp.max(jnp.sum(aq, axis=1), axis=0))
                for rb in range(4):
                    for gg in range(4):
                        k_limbs(pl.multiple_of(r0 + rb * 32, 32), gg, beta8)
            return bound
        bound = jax.lax.fori_loop(0, S // TA2, qproj, jnp.zeros((8, 128), f32))

        def vproj(t, _):
            p_c[...] = jnp.zeros(p_c.shape, f32)
            acc_c[...] = jnp.zeros(acc_c.shape, f32)
            l_c[...] = jnp.ones(l_c.shape, f32)
            v_c[1, S // TK - 1] = jnp.zeros((8, 128), i32)
            for cc in range(TA2 // 128):
                ct = t * (TA2 // 128) + cc
                r0 = pl.multiple_of(ct * 128, 128)
                xn = _wide(xns, pl.ds(r0, 128))
                for o in range(4):
                    rows = slice(o * 128, (o + 1) * 128)
                    wv = pltpu.bitcast(wvT[o * 64:(o + 1) * 64, :], bf16)
                    v = jax.lax.dot_general(wv, xn, NT, preferred_element_type=f32)
                    vT[ct, rows, :] = v.astype(bf16)
                    for k in range(4):
                        q_limbs(ct, o, k)
            return jnp.max(bound)
        bmax = jax.lax.fori_loop(0, S // TA2, vproj, jnp.float32(0))
        safe = (bmax * (SCALE * LOG2E) < SAFE_LOG2) & v_ok

        def o_transpose(t):
            on = oT[:, pl.ds(_aligned(t * TM, TM), TS)].T
            for j in range(ND):
                oN[j] = on[:, j * 128:(j + 1) * 128]

        @pl.when(safe)
        def _fast():
            nq = S // TQ
            nk = S // TK
            cq = TQ // 128

            def head_of(g, b):
                return ((g >> 2) << 3) + 4 * b + (g & 3)

            def pv(v, pb, acc):
                return acc + jnp.dot(pltpu.bitcast(v, bf16), pb, preferred_element_type=f32)

            def finish(h, q0, acc, ls):
                lsum = jnp.sum(ls, axis=0, keepdims=True)
                r = pl.reciprocal(lsum, approx=True)
                r = r * (2.0 - lsum * r)
                oT[pl.ds(_aligned(h * DH, DH), DH), pl.ds(q0, TQ)] = (acc * r).astype(bf16)

            def body(g, _):
                ph, pq0 = head_of(jnp.maximum(g - 1, 0), 1), (nq - 1) * TQ
                pb, acc, pls = p_c[...].astype(bf16), acc_c[0], l_c[...]
                pv_last = v_c[1, nk - 1]
                k_c[...] = pltpu.roll(pltpu.bitcast(kl[g], i32), 64, 1)
                for b in range(2):
                    h = head_of(g, b)
                    for kc in range(nk):
                        v_c[b, kc] = pltpu.bitcast(
                            vT[kc, pl.ds(_aligned(h * DH, DH), DH), :], i32)
                    for j in range(NC):
                        c_c[b, :, j * 128:(j + 1) * 128] = jnp.broadcast_to(
                            cs[j, pl.ds(h, 1), :], (8, 128))
                zero = jnp.zeros((DH, TQ), i32)
                for qt in range(nq):
                    for b in range(2):
                        h = head_of(g, b)
                        words = jnp.concatenate(
                            [qw[qt * cq + j, pl.ds(h, DH, stride=QS), :] for j in range(cq)],
                            axis=1)
                        w = pltpu.bitcast(jnp.concatenate([words, zero], axis=0), i8)
                        c = c_c[b, :, qt * TQ:(qt + 1) * TQ]
                        ls = None
                        for kc in range(nk):
                            if b == 0:
                                kk = kl[g, kc * TK:(kc + 1) * TK, :]
                            else:
                                kk = pltpu.bitcast(
                                    k_c[kc * (TK // 4):(kc + 1) * (TK // 4), :], i8)
                            s = jnp.dot(kk, w, preferred_element_type=i32)
                            if kc == 0:
                                finish(ph, pq0, pv(pv_last, pb, acc), pls)
                                acc = acc_c[1]
                            else:
                                acc = pv(v_c[b, kc - 1], pb, acc)
                            p = jnp.exp2(s.astype(f32).reshape(TK // 8, 8, TQ) * c)
                            psum = jnp.sum(p, axis=0)
                            ls = psum if ls is None else ls + psum
                            p = p.reshape(TK, TQ)
                            pb = p.astype(bf16)
                        ph, pq0, pls, pv_last = h, qt * TQ, ls, v_c[b, nk - 1]
                p_c[...] = p
                acc_c[0] = acc
                l_c[...] = pls
                return 0
            jax.lax.fori_loop(0, NG, body, 0)
            o_transpose(0)
            finish(H - 1, (nq - 1) * TQ,
                   pv(v_c[1, nk - 1], p_c[...].astype(bf16), acc_c[0]), l_c[...])

        @pl.when(jnp.logical_not(safe))
        def _slow():
            def qraw(ct, _):
                qT[ct, 0:D, :] = q_raw(pl.multiple_of(ct * 128, 128))
                return 0
            jax.lax.fori_loop(0, NC, qraw, 0)

            def body(i, _):
                h = i // NC
                ct = i % NC
                q0 = pl.multiple_of(ct * 128, 128)
                g0 = pl.multiple_of((h // 8) * 128, 128)
                r0 = pl.multiple_of(h * DH, DH)
                qh = qT[ct, pl.ds(g0 + h % 8, DH, stride=8), :]
                row = jax.lax.broadcasted_iota(i32, (128, 128), 0)
                w = jnp.where(row // DH == h % 8, jnp.concatenate([qh] * 8, axis=0), 0.0)
                kb = kf[:, pl.ds(g0, 128)].astype(bf16)
                s = jnp.dot(kb, w.astype(bf16), preferred_element_type=f32) * SCALE
                m = jnp.max(s, axis=0, keepdims=True)
                p = jnp.exp(s - m)
                lsum = jnp.sum(p, axis=0, keepdims=True)
                acc = jnp.dot(_wide(vT, pl.ds(r0, DH)), p.astype(bf16),
                              preferred_element_type=f32)
                oT[pl.ds(r0, DH), pl.ds(q0, 128)] = (acc / lsum).astype(bf16)
                return 0
            jax.lax.fori_loop(0, H * NC, body, 0)
            o_transpose(0)

        def ffn(t, last):
            ns = TM // TS
            rs = [pl.multiple_of(t * TM + u * TS, TS) for u in range(ns)]
            b1 = b1f[...]
            b2 = b2f[...]
            x0 = [(xs if last else xb)[pl.ds(r, TS), :].astype(f32) for r in rs]
            x1 = [x0[0] + jnp.dot(_wide(oN), wo[...], preferred_element_type=f32)]
            x1 += [x + jax.lax.dot_general(
                oT[:, pl.ds(r, TS)], wo[...], TN, preferred_element_type=f32)
                for r, x in zip(rs[1:], x0[1:])]
            o_transpose(jnp.minimum(t + 1, S // TM - 1))
            hh = [_gelu(jnp.dot(_layernorm(x).astype(bf16), w1[...],
                                preferred_element_type=f32) + b1).astype(bf16) for x in x1]
            x2 = []
            for u, (r, x, g) in enumerate(zip(rs, x1, hh)):
                x = x + jnp.dot(g, w2[...], preferred_element_type=f32) + b2
                if last:
                    xb[pl.ds(r, TS), :] = x.astype(bf16)
                    out_copy(t * ns + u).start()
                else:
                    xs[pl.ds(r, TS), :] = x
                    x2.append(x)
            if not last:
                km = kmx[...]
                for r, x in zip(rs, x2):
                    km = jnp.maximum(km, k_proj(ln_store(x, r, TS), r, TS))
                kmx[...] = km
            return 0

        @pl.when(li == 0)
        def _():
            for cp in late:
                cp.wait()
            b1f[...] = b1v[...].astype(f32).reshape(1, F)
            b2f[...] = b2v[...].astype(f32).reshape(1, D)

        @pl.when(li < N_LAYERS - 1)
        def _():
            kmx[...] = jnp.zeros(kmx.shape, f32)
            jax.lax.fori_loop(0, S // TM, lambda t, _: ffn(t, False), 0)

        @pl.when(li == N_LAYERS - 1)
        def _():
            jax.lax.fori_loop(0, S // TM, lambda t, _: ffn(t, True), 0)
        return carry

    jax.lax.fori_loop(0, N_LAYERS, layer, 0)
    for u in range(S // TS):
        out_copy(u).wait()


@jax.jit
def pallas_interleave_layers__mha_block__dense_activation_gelu__prompt_kernel(
    A_x: jax.Array,
    A_wqkv: jax.Array,
    A_wo: jax.Array,
    B_x: jax.Array,
    B_w1: jax.Array,
    B_b1: jax.Array,
    B_w2: jax.Array,
    B_b2: jax.Array,
):
    del B_x
    hbm = pl.BlockSpec(memory_space=pl.ANY)
    out = pl.pallas_call(
        _kernel,
        out_shape=jax.ShapeDtypeStruct((S, D), A_x.dtype),
        in_specs=[hbm] * 7,
        out_specs=hbm,
        scratch_shapes=[
            pltpu.VMEM((S, D), bf16),
            pltpu.VMEM((3, D, D), bf16),
            pltpu.VMEM((D, D), bf16),
            pltpu.VMEM((D, F), bf16),
            pltpu.VMEM((F, D), bf16),
            pltpu.SemaphoreType.DMA((NX + 5,)),
            pltpu.VMEM((S, D), f32),
            pltpu.VMEM((ND, S, 128), bf16),
            pltpu.VMEM((D // 2, D), i32),
            pltpu.VMEM((D // 2, D), i32),
            pltpu.VMEM((ND, (H + 1) * HS, 128), f32),
            pltpu.VMEM((S, D), f32),
            pltpu.VMEM((8, D), f32),
            pltpu.VMEM((NC, D + 8, 128), f32),
            pltpu.VMEM((NC, D, 128), bf16),
            pltpu.VMEM((NG, S, 128), i8),
            pltpu.VMEM((NC, (DH + 1) * QS, 128), i32),
            pltpu.VMEM((NC, H, 128), f32),
            pltpu.VMEM((NC, H, 128), f32),
            pltpu.VMEM((D, S), bf16),
            pltpu.VMEM((ND, TS, 128), bf16),
            pltpu.VMEM((TK, TQ), f32),
            pltpu.VMEM((2, DH, TQ), f32),
            pltpu.VMEM((8, TQ), f32),
            pltpu.VMEM((S // 4, 128), i32),
            pltpu.VMEM((2, NC, 8, 128), i32),
            pltpu.VMEM((2, 8, S), f32),
            pltpu.VMEM((8, 8, 128), f32),
            pltpu.VMEM((F,), bf16),
            pltpu.VMEM((D,), bf16),
            pltpu.VMEM((1, F), f32),
            pltpu.VMEM((1, D), f32),
        ],
        compiler_params=pltpu.CompilerParams(vmem_limit_bytes=100 * 1024 * 1024),
    )(A_x.reshape(S, D), A_wqkv, A_wo, B_w1, B_b1, B_w2, B_b2)
    return out.reshape(1, S, D)
```

```python
import jax
import jax.numpy as jnp
import jax.experimental.pallas as pl
import jax.experimental.pallas.tpu as pltpu

S, D, H, DH, F = 2048, 512, 32, 16, 1792
N_LAYERS = 2
EPS = 1e-5
LOG2E = 1.4426950408889634
SCALE = DH ** -0.5
MAGIC = 12582912.0

SIGN_BYTES = 0x80808080 - 2 ** 32

NG = H // 2
NC = S // 128
ND = D // 128
X_CHUNKS = ((0, 256), (256, 256), (512, 768), (1280, 768))
NX = len(X_CHUNKS)
TA = 256
W_AT = 4
TA2 = 1024
TM = 256
TS = 128
TQ = 1024
PAIRS = 2
TK = 128
TIE_ROW = 88
HS = 24
QS = 40

SAFE_LOG2 = 64.0
WV_MIN, WV_MAX = 2.0 ** -20, 2.0 ** 20

bf16 = jnp.bfloat16
f32 = jnp.float32
i32 = jnp.int32
i8 = jnp.int8
NT = (((1,), (1,)), ((), ()))
TN = (((0,), (0,)), ((), ()))


def _layernorm(x):
    m = jnp.mean(x, axis=-1, keepdims=True)
    xc = x - m
    v = jnp.mean(xc * xc, axis=-1, keepdims=True)
    return xc * jax.lax.rsqrt(v + EPS)


def _gelu(x):
    c = 0.7978845608028654
    return 0.5 * x * (1.0 + jnp.tanh(c * (x + 0.044715 * (x * x * x))))


def _bits(t):
    return pltpu.bitcast(t, i32)


PACKS = ((0, 256), (1, 128), (4, 128), (-4, 16 * 256 + 128))
BIG = 2.0 ** 31 + 2.0 ** 21


def _pack_consts(e, off):
    return [(BIG - 2.0 ** 23 - 257 * off - extra) * 2.0 ** e
            for extra in (0, 2 ** 16 - ((150 + e) << 7))]


def _pack_rounded(x, e, sub):
    def pair(lo, hi256, c):
        return _bits(((hi256 + BIG * 2.0 ** e) - c) + lo)
    return pair(x[0], x[1], sub[0]) + (pair(x[2], x[3], sub[1]) << 16)


def _wide(ref, rows=slice(None)):
    return jnp.concatenate([ref[j, rows, :] for j in range(ref.shape[0])], axis=1)


def _aligned(i, n):
    return i if isinstance(i, int) else pl.multiple_of(i, n)


def _kernel(x_hbm, wqkv_hbm, wo_hbm, w1_hbm, b1_hbm, w2_hbm, b2_hbm, o_hbm,
            xb, wqkv, wo, w1, w2, sems,
            xs, xns, wqT, wvT, tmp, kf, kmx, qT, vT, kl, qw, cs, al, oT, oN,
            p_c, acc_c, l_c, k_c, v_c, c_c, cst, b1v, b2v, b1f, b2f):

    def x_copy(c):
        r0, n = X_CHUNKS[c]
        return pltpu.make_async_copy(x_hbm.at[pl.ds(r0, n), :], xb.at[pl.ds(r0, n), :],
                                     sems.at[c])

    def wqkv_copy(j):
        return pltpu.make_async_copy(wqkv_hbm.at[:, pl.ds(j * D, D)], wqkv.at[j],
                                     sems.at[NX + j])

    late = [pltpu.make_async_copy(src, dst, sems.at[NX + 3]) for src, dst in
            ((wo_hbm, wo), (w1_hbm, w1), (w2_hbm, w2), (b1_hbm, b1v), (b2_hbm, b2v))]

    def out_copy(u):
        r0 = _aligned(u * TS, TS)
        return pltpu.make_async_copy(xb.at[pl.ds(r0, TS), :], o_hbm.at[pl.ds(r0, TS), :],
                                     sems.at[NX + 4])

    x_copy(0).start()
    wqkv_copy(1).start()
    for c in range(1, NX):
        x_copy(c).start()
    wqkv_copy(0).start()
    wqkv_copy(2).start()
    for cp in late:
        cp.start()

    for i, (e, off) in enumerate(PACKS):
        for j, c in enumerate(_pack_consts(e, off)):
            cst[2 * i + j] = jnp.full((8, 128), c, f32)

    for ct in range(NC):
        for j in range(DH):
            qw[ct, j * QS + H:(j + 1) * QS, :] = jnp.zeros((QS - H, 128), i32)
        qw[ct, DH * QS:, :] = jnp.zeros((QS, 128), i32)
        qT[ct, D:, :] = jnp.zeros((8, 128), f32)
    for j in range(ND):
        for h in range(H):
            tmp[j, h * HS + DH:(h + 1) * HS, :] = jnp.zeros((HS - DH, 128), f32)
        tmp[j, H * HS:, :] = jnp.zeros((HS, 128), f32)

    def ln_store(x, r0, n):
        xn = _layernorm(x).astype(bf16)
        for j in range(ND):
            xns[j, pl.ds(r0, n), :] = xn[:, j * 128:(j + 1) * 128]
        return xn

    def k_proj(xn, r0, n):
        k = jnp.dot(xn, wqkv[1], preferred_element_type=f32)
        kf[pl.ds(r0, n), :] = k
        return jnp.max(jnp.abs(k).reshape(n // 8, 8, D), axis=0)

    def first_ln(u):
        ln_store(xb[u * TA:(u + 1) * TA, :].astype(f32), u * TA, TA)

    def w_transposes(j):
        cols = slice(j * 128, (j + 1) * 128)
        wv = wqkv[2, cols, :]
        wvT[:, cols] = pltpu.bitcast(wv.T, i32)
        wq_t = wqkv[0, cols, :].T.astype(f32)
        for h in range(H):
            tmp[j, h * HS:h * HS + DH, :] = wq_t[h * DH:(h + 1) * DH]
        for o in range(4):
            for d2 in range(DH // 2):
                r = o * 64 + d2 * 8
                wqT[r:r + 8, cols] = pltpu.bitcast(jnp.concatenate(
                    [tmp[j, pl.ds(o * 8 * HS + 2 * d2 + e, 8, stride=HS), :]
                     for e in range(2)], axis=0).astype(bf16), i32)
        return jnp.max(jnp.abs(wv.astype(f32)).reshape(16, 8, D), axis=0)

    x_copy(0).wait()
    first_ln(0)
    kmax8 = jnp.zeros((8, D), f32)
    wv_max = jnp.zeros((8, D), f32)
    starts = {r0 // TA: c for c, (r0, _) in enumerate(X_CHUNKS)}
    for u in range(S // TA):
        if u == 0:
            wqkv_copy(1).wait()
        if u + 1 in starts:
            x_copy(starts[u + 1]).wait()
        if u == W_AT:
            wqkv_copy(0).wait()
            wqkv_copy(2).wait()
        if u >= W_AT:
            wv_max = jnp.maximum(wv_max, w_transposes(u - W_AT))
        kmax8 = jnp.maximum(kmax8, k_proj(_wide(xns, slice(u * TA, (u + 1) * TA)), u * TA, TA))
        if u + 1 < S // TA:
            first_ln(u + 1)
    kmx[...] = kmax8
    wv_max = jnp.max(wv_max)
    v_ok = (wv_max >= WV_MIN) & (wv_max <= WV_MAX)

    def layer(li, carry):
        def k_stats():
            kmax = jnp.maximum(jnp.max(kmx[...], axis=0, keepdims=True), 1e-30)
            kc = jnp.broadcast_to(kmax, (128, D)).T
            for h in range(H):
                tmp[0, h * HS:h * HS + DH, :] = kc[h * DH:(h + 1) * DH]
            for o in range(4):
                for d in range(DH):
                    r = o * 128 + d * 8
                    tmp[1, r:r + 8, :] = tmp[0, pl.ds(o * 8 * HS + d, 8, stride=HS), :]
            return jnp.broadcast_to(127.0 / kmax, (8, D))

        def k_limbs(r0, gg, beta8):
            seg = (jax.lax.broadcasted_iota(i32, (8, 128), 1) // DH) % 4
            y = kf[pl.ds(r0, 32), gg * 128:(gg + 1) * 128].reshape(4, 8, 128) \
                * beta8[:, gg * 128:(gg + 1) * 128]
            t0 = _bits(y + MAGIC)
            te = _bits(y + MAGIC / 16) - (t0 << 4)
            t1 = _bits(y + MAGIC * 16)
            y0, ey, y1 = [pltpu.bitcast(a.reshape(32, 128).astype(i8), i32)
                          for a in (t0, te, t1)]

            def rolled(a, k):
                return a if k == 0 else pltpu.roll(a, (DH * k) % 128, 1)
            ry0 = {k: rolled(y0, k) for k in range(-3, 2)}
            rey = {k: rolled(ey, k) for k in range(-1, 3)}
            ry1 = {k: rolled(y1, k) for k in range(0, 4)}
            for r in range(4):
                out = jnp.where(seg < 2,
                                jnp.where(seg == 0, ry0[0 - r], ry0[1 - r]),
                                jnp.where(seg == 2, rey[2 - r], ry1[3 - r]))
                kl[gg * 4 + r, pl.ds(r0, 32), :] = pltpu.bitcast(out, i8)

        def q_limbs(ct, o, k):
            r = o * 128 + k * 32
            q = qT[ct, r:r + 32, :].reshape(4, 8, 128)
            a1 = al[ct, o * 8:(o + 1) * 8, :]
            a256 = a1 * 256.0
            x = (q[0] * a1, q[1] * a256, q[2] * a1, q[3] * a256)
            w0, u, x1, w16 = [_pack_rounded(x, e, (cst[2 * i], cst[2 * i + 1]))
                              for i, (e, _) in enumerate(PACKS)]
            for j, word in enumerate((u, w0 - u, x1, w16 - (w0 << 4))):
                r = (4 * j + k) * QS + o * 8
                qw[ct, r:r + 8, :] = word ^ SIGN_BYTES

        def q_raw(r0):
            return jax.lax.dot_general(pltpu.bitcast(wqT[...], bf16), _wide(xns, pl.ds(r0, 128)),
                                       NT, preferred_element_type=f32)

        beta8 = k_stats()
        bound = jnp.zeros((8, 128), f32)
        for ct in range(NC):
            r0 = ct * 128
            q = q_raw(r0) * tmp[1, 0:D, :]
            qT[ct, 0:D, :] = q
            aq = jnp.abs(q).reshape(4, DH, 8, 128)
            amax = jnp.maximum(jnp.max(aq, axis=1), 1e-30).reshape(H, 128)
            al[ct] = 254.0 / amax
            cs[ct] = amax * (SCALE * LOG2E / (254.0 * 127.0))
            bound = jnp.maximum(bound, jnp.max(jnp.sum(aq, axis=1), axis=0))
            for rb in range(4):
                for gg in range(4):
                    k_limbs(r0 + rb * 32, gg, beta8)

        def vproj(t, _):
            p_c[...] = jnp.zeros(p_c.shape, f32)
            acc_c[...] = jnp.zeros(acc_c.shape, f32)
            l_c[...] = jnp.ones(l_c.shape, f32)
            v_c[2 * PAIRS - 1, S // TK - 1] = jnp.zeros((8, 128), i32)
            for cc in range(TA2 // 128):
                ct = t * (TA2 // 128) + cc
                r0 = pl.multiple_of(ct * 128, 128)
                xn = _wide(xns, pl.ds(r0, 128))
                for o in range(4):
                    rows = slice(o * 128, (o + 1) * 128)
                    wv = pltpu.bitcast(wvT[o * 64:(o + 1) * 64, :], bf16)
                    v = jax.lax.dot_general(wv, xn, NT, preferred_element_type=f32)
                    vT[ct, rows, :] = v.astype(bf16)
                    for k in range(4):
                        q_limbs(ct, o, k)
            return jnp.max(bound)
        bmax = jax.lax.fori_loop(0, S // TA2, vproj, jnp.float32(0))
        safe = (bmax * (SCALE * LOG2E) < SAFE_LOG2) & v_ok

        def o_transpose(r0):
            on = oT[:, pl.ds(_aligned(r0, TS), TS)].T
            for j in range(ND):
                oN[j] = on[:, j * 128:(j + 1) * 128]

        @pl.when(safe)
        def _fast():
            nq = S // TQ
            nk = S // TK
            cq = TQ // 128

            def head_of(g, b):
                return ((g >> 2) << 3) + 4 * b + (g & 3)

            def pv(v, p, acc, s=None):
                zi = pltpu.bitcast(acc_c[1, 0:8, 0:128], i32)
                outs = []
                for t in range(cq):
                    vt = v
                    if s is not None and t in (2, 3):
                        vt = v | (s[TIE_ROW:TIE_ROW + 8, (t - 2) * 128:(t - 1) * 128] & zi)
                    outs.append(jnp.dot(pltpu.bitcast(vt, bf16),
                                        p[:, t * 128:(t + 1) * 128].astype(bf16),
                                        preferred_element_type=f32))
                return acc + jnp.concatenate(outs, axis=1)

            def finish(h, q0, acc, ls):
                lsum = jnp.sum(ls, axis=0, keepdims=True)
                r = pl.reciprocal(lsum, approx=True)
                r = r * (2.0 - lsum * r)
                oT[pl.ds(_aligned(h * DH, DH), DH), pl.ds(q0, TQ)] = (acc * r).astype(bf16)

            def body(i, _):
                ph, pq0 = head_of(jnp.maximum(i * PAIRS - 1, 0), 1), (nq - 1) * TQ
                p, acc, pls = p_c[...], acc_c[0], l_c[...]
                pv_last = v_c[2 * PAIRS - 1, nk - 1]
                zero = jnp.zeros((DH, TQ), i32)
                for gi in range(PAIRS):
                    g = i * PAIRS + gi
                    k_c[gi] = pltpu.roll(pltpu.bitcast(kl[g], i32), 64, 1)
                    for b in range(2):
                        h = head_of(g, b)
                        for kc in range(nk):
                            v_c[2 * gi + b, kc] = pltpu.bitcast(
                                vT[kc, pl.ds(_aligned(h * DH, DH), DH), :], i32)
                        for j in range(NC):
                            c_c[2 * gi + b, :, j * 128:(j + 1) * 128] = jnp.broadcast_to(
                                cs[j, pl.ds(h, 1), :], (8, 128))
                    for qt in range(nq):
                        for b in range(2):
                            h = head_of(g, b)
                            n = 2 * gi + b
                            words = jnp.concatenate(
                                [qw[qt * cq + j, pl.ds(h, DH, stride=QS), :] for j in range(cq)],
                                axis=1)
                            w = pltpu.bitcast(jnp.concatenate([words, zero], axis=0), i8)
                            c = c_c[n, :, qt * TQ:(qt + 1) * TQ]
                            ls = None
                            for kc in range(nk):
                                if b == 0:
                                    kk = kl[g, kc * TK:(kc + 1) * TK, :]
                                else:
                                    kk = pltpu.bitcast(
                                        k_c[gi, kc * (TK // 4):(kc + 1) * (TK // 4), :], i8)
                                s = jnp.dot(kk, w, preferred_element_type=i32)
                                if kc == 0:
                                    finish(ph, pq0, pv(pv_last, p, acc, s), pls)
                                    acc = acc_c[1]
                                else:
                                    acc = pv(v_c[n, kc - 1], p, acc, s)
                                p = jnp.exp2(s.astype(f32).reshape(TK // 8, 8, TQ) * c)
                                psum = jnp.sum(p, axis=0)
                                ls = psum if ls is None else ls + psum
                                p = p.reshape(TK, TQ)
                            ph, pq0, pls, pv_last = h, qt * TQ, ls, v_c[n, nk - 1]
                p_c[...] = p
                acc_c[0] = acc
                l_c[...] = pls
                return 0
            jax.lax.fori_loop(0, NG // PAIRS, body, 0)
            o_transpose(0)
            finish(H - 1, (nq - 1) * TQ,
                   pv(v_c[2 * PAIRS - 1, nk - 1], p_c[...], acc_c[0]), l_c[...])

        @pl.when(jnp.logical_not(safe))
        def _slow():
            def qraw(ct, _):
                qT[ct, 0:D, :] = q_raw(pl.multiple_of(ct * 128, 128))
                return 0
            jax.lax.fori_loop(0, NC, qraw, 0)

            def body(i, _):
                h = i // NC
                ct = i % NC
                q0 = pl.multiple_of(ct * 128, 128)
                g0 = pl.multiple_of((h // 8) * 128, 128)
                r0 = pl.multiple_of(h * DH, DH)
                qh = qT[ct, pl.ds(g0 + h % 8, DH, stride=8), :]
                row = jax.lax.broadcasted_iota(i32, (128, 128), 0)
                w = jnp.where(row // DH == h % 8, jnp.concatenate([qh] * 8, axis=0), 0.0)
                kb = kf[:, pl.ds(g0, 128)].astype(bf16)
                s = jnp.dot(kb, w.astype(bf16), preferred_element_type=f32) * SCALE
                m = jnp.max(s, axis=0, keepdims=True)
                p = jnp.exp(s - m)
                lsum = jnp.sum(p, axis=0, keepdims=True)
                acc = jnp.dot(_wide(vT, pl.ds(r0, DH)), p.astype(bf16),
                              preferred_element_type=f32)
                oT[pl.ds(r0, DH), pl.ds(q0, 128)] = (acc / lsum).astype(bf16)
                return 0
            jax.lax.fori_loop(0, H * NC, body, 0)
            o_transpose(0)

        def ffn(t, last):
            ns = TM // TS
            rs = [pl.multiple_of(t * TM + u * TS, TS) for u in range(ns)]
            b1 = b1f[...]
            b2 = b2f[...]
            x0 = [(xs if last else xb)[pl.ds(r, TS), :].astype(f32) for r in rs]
            x1 = [x0[0] + jnp.dot(_wide(oN), wo[...], preferred_element_type=f32)]
            x1 += [x + jax.lax.dot_general(
                oT[:, pl.ds(r, TS)], wo[...], TN, preferred_element_type=f32)
                for r, x in zip(rs[1:], x0[1:])]
            o_transpose(jnp.minimum(t + 1, S // TM - 1) * TM)
            hh = [_gelu(jnp.dot(_layernorm(x).astype(bf16), w1[...],
                                preferred_element_type=f32) + b1).astype(bf16) for x in x1]
            x2 = []
            for u, (r, x, g) in enumerate(zip(rs, x1, hh)):
                x = x + jnp.dot(g, w2[...], preferred_element_type=f32) + b2
                if last:
                    xb[pl.ds(r, TS), :] = x.astype(bf16)
                    out_copy(t * ns + u).start()
                else:
                    xs[pl.ds(r, TS), :] = x
                    x2.append(x)
            if not last:
                km = kmx[...]
                for r, x in zip(rs, x2):
                    km = jnp.maximum(km, k_proj(ln_store(x, r, TS), r, TS))
                kmx[...] = km
            return 0

        @pl.when(li == 0)
        def _():
            for cp in late:
                cp.wait()
            b1f[...] = b1v[...].astype(f32).reshape(1, F)
            b2f[...] = b2v[...].astype(f32).reshape(1, D)

        @pl.when(li < N_LAYERS - 1)
        def _():
            kmx[...] = jnp.zeros(kmx.shape, f32)
            jax.lax.fori_loop(0, S // TM, lambda t, _: ffn(t, False), 0)

        @pl.when(li == N_LAYERS - 1)
        def _():
            jax.lax.fori_loop(0, S // TM, lambda t, _: ffn(t, True), 0)
        return carry

    jax.lax.fori_loop(0, N_LAYERS, layer, 0)
    for u in range(S // TS):
        out_copy(u).wait()


@jax.jit
def pallas_interleave_layers__mha_block__dense_activation_gelu__prompt_kernel(
    A_x: jax.Array,
    A_wqkv: jax.Array,
    A_wo: jax.Array,
    B_x: jax.Array,
    B_w1: jax.Array,
    B_b1: jax.Array,
    B_w2: jax.Array,
    B_b2: jax.Array,
):
    del B_x
    hbm = pl.BlockSpec(memory_space=pl.ANY)
    out = pl.pallas_call(
        _kernel,
        out_shape=jax.ShapeDtypeStruct((S, D), A_x.dtype),
        in_specs=[hbm] * 7,
        out_specs=hbm,
        scratch_shapes=[
            pltpu.VMEM((S, D), bf16),
            pltpu.VMEM((3, D, D), bf16),
            pltpu.VMEM((D, D), bf16),
            pltpu.VMEM((D, F), bf16),
            pltpu.VMEM((F, D), bf16),
            pltpu.SemaphoreType.DMA((NX + 5,)),
            pltpu.VMEM((S, D), f32),
            pltpu.VMEM((ND, S, 128), bf16),
            pltpu.VMEM((D // 2, D), i32),
            pltpu.VMEM((D // 2, D), i32),
            pltpu.VMEM((ND, (H + 1) * HS, 128), f32),
            pltpu.VMEM((S, D), f32),
            pltpu.VMEM((8, D), f32),
            pltpu.VMEM((NC, D + 8, 128), f32),
            pltpu.VMEM((NC, D, 128), bf16),
            pltpu.VMEM((NG, S, 128), i8),
            pltpu.VMEM((NC, (DH + 1) * QS, 128), i32),
            pltpu.VMEM((NC, H, 128), f32),
            pltpu.VMEM((NC, H, 128), f32),
            pltpu.VMEM((D, S), bf16),
            pltpu.VMEM((ND, TS, 128), bf16),
            pltpu.VMEM((TK, TQ), f32),
            pltpu.VMEM((2, DH, TQ), f32),
            pltpu.VMEM((8, TQ), f32),
            pltpu.VMEM((PAIRS, S // 4, 128), i32),
            pltpu.VMEM((2 * PAIRS, NC, 8, 128), i32),
            pltpu.VMEM((2 * PAIRS, 8, S), f32),
            pltpu.VMEM((8, 8, 128), f32),
            pltpu.VMEM((F,), bf16),
            pltpu.VMEM((D,), bf16),
            pltpu.VMEM((1, F), f32),
            pltpu.VMEM((1, D), f32),
        ],
        compiler_params=pltpu.CompilerParams(vmem_limit_bytes=100 * 1024 * 1024),
    )(A_x.reshape(S, D), A_wqkv, A_wo, B_w1, B_b1, B_w2, B_b2)
    return out.reshape(1, S, D)
```

```python
import jax
import jax.numpy as jnp
import jax.experimental.pallas as pl
import jax.experimental.pallas.tpu as pltpu

S, D, H, DH, F = 2048, 512, 32, 16, 1792
N_LAYERS = 2
EPS = 1e-5
LOG2E = 1.4426950408889634
SCALE = DH ** -0.5
MAGIC = 12582912.0

SIGN_BYTES = 0x80808080 - 2 ** 32

NG = H // 2
NC = S // 128
ND = D // 128
X_CHUNKS = ((0, 256), (256, 256), (512, 768), (1280, 768))
NX = len(X_CHUNKS)
TA = 256
W_AT = 4
TA2 = 1024
TM = 256
TS = 128
TQ = 1024
PAIRS = 2
TK = 128
TIE_ROW = 40
HS = 24
QS = 40

SAFE_LOG2 = 64.0
WV_MIN, WV_MAX = 2.0 ** -20, 2.0 ** 20

bf16 = jnp.bfloat16
f32 = jnp.float32
i32 = jnp.int32
i8 = jnp.int8
NT = (((1,), (1,)), ((), ()))
TN = (((0,), (0,)), ((), ()))


def _layernorm(x):
    m = jnp.mean(x, axis=-1, keepdims=True)
    xc = x - m
    v = jnp.mean(xc * xc, axis=-1, keepdims=True)
    return xc * jax.lax.rsqrt(v + EPS)


def _gelu(x):
    c = 0.7978845608028654
    return 0.5 * x * (1.0 + jnp.tanh(c * (x + 0.044715 * (x * x * x))))


def _bits(t):
    return pltpu.bitcast(t, i32)


PACKS = ((0, 256), (1, 128), (4, 128), (-4, 16 * 256 + 128))
BIG = 2.0 ** 31 + 2.0 ** 21


def _pack_consts(e, off):
    return [(BIG - 2.0 ** 23 - 257 * off - extra) * 2.0 ** e
            for extra in (0, 2 ** 16 - ((150 + e) << 7))]


def _pack_rounded(x, e, sub):
    def pair(lo, hi256, c):
        return _bits(((hi256 + BIG * 2.0 ** e) - c) + lo)
    return pair(x[0], x[1], sub[0]) + (pair(x[2], x[3], sub[1]) << 16)


def _wide(ref, rows=slice(None)):
    return jnp.concatenate([ref[j, rows, :] for j in range(ref.shape[0])], axis=1)


def _aligned(i, n):
    return i if isinstance(i, int) else pl.multiple_of(i, n)


def _kernel(x_hbm, wqkv_hbm, wo_hbm, w1_hbm, b1_hbm, w2_hbm, b2_hbm, o_hbm,
            xb, wqkv, wo, w1, w2, sems,
            xs, xns, wqT, wvT, tmp, kf, kmx, qT, vT, kl, qw, cs, al, oT, oN,
            p_c, acc_c, l_c, k_c, v_c, c_c, cst, b1v, b2v, b1f, b2f):

    def x_copy(c):
        r0, n = X_CHUNKS[c]
        return pltpu.make_async_copy(x_hbm.at[pl.ds(r0, n), :], xb.at[pl.ds(r0, n), :],
                                     sems.at[c])

    def wqkv_copy(j):
        return pltpu.make_async_copy(wqkv_hbm.at[:, pl.ds(j * D, D)], wqkv.at[j],
                                     sems.at[NX + j])

    late = [pltpu.make_async_copy(src, dst, sems.at[NX + 3]) for src, dst in
            ((wo_hbm, wo), (w1_hbm, w1), (w2_hbm, w2), (b1_hbm, b1v), (b2_hbm, b2v))]

    def out_copy(u):
        r0 = _aligned(u * TS, TS)
        return pltpu.make_async_copy(xb.at[pl.ds(r0, TS), :], o_hbm.at[pl.ds(r0, TS), :],
                                     sems.at[NX + 4])

    x_copy(0).start()
    wqkv_copy(1).start()
    for c in range(1, NX):
        x_copy(c).start()
    wqkv_copy(0).start()
    wqkv_copy(2).start()
    for cp in late:
        cp.start()

    for i, (e, off) in enumerate(PACKS):
        for j, c in enumerate(_pack_consts(e, off)):
            cst[2 * i + j] = jnp.full((8, 128), c, f32)

    for ct in range(NC):
        for j in range(DH):
            qw[ct, j * QS + H:(j + 1) * QS, :] = jnp.zeros((QS - H, 128), i32)
        qw[ct, DH * QS:, :] = jnp.zeros((QS, 128), i32)
        qT[ct, D:, :] = jnp.zeros((8, 128), f32)
    for j in range(ND):
        for h in range(H):
            tmp[j, h * HS + DH:(h + 1) * HS, :] = jnp.zeros((HS - DH, 128), f32)
        tmp[j, H * HS:, :] = jnp.zeros((HS, 128), f32)

    def ln_store(x, r0, n):
        xn = _layernorm(x).astype(bf16)
        for j in range(ND):
            xns[j, pl.ds(r0, n), :] = xn[:, j * 128:(j + 1) * 128]
        return xn

    def k_proj(xn, r0, n):
        k = jnp.dot(xn, wqkv[1], preferred_element_type=f32)
        kf[pl.ds(r0, n), :] = k
        return jnp.max(jnp.abs(k).reshape(n // 8, 8, D), axis=0)

    def first_ln(u):
        ln_store(xb[u * TA:(u + 1) * TA, :].astype(f32), u * TA, TA)

    def w_transposes(j):
        cols = slice(j * 128, (j + 1) * 128)
        wv = wqkv[2, cols, :]
        wvT[:, cols] = pltpu.bitcast(wv.T, i32)
        wq_t = wqkv[0, cols, :].T.astype(f32)
        for h in range(H):
            tmp[j, h * HS:h * HS + DH, :] = wq_t[h * DH:(h + 1) * DH]
        for o in range(4):
            for d2 in range(DH // 2):
                r = o * 64 + d2 * 8
                wqT[r:r + 8, cols] = pltpu.bitcast(jnp.concatenate(
                    [tmp[j, pl.ds(o * 8 * HS + 2 * d2 + e, 8, stride=HS), :]
                     for e in range(2)], axis=0).astype(bf16), i32)
        return jnp.max(jnp.abs(wv.astype(f32)).reshape(16, 8, D), axis=0)

    x_copy(0).wait()
    first_ln(0)
    kmax8 = jnp.zeros((8, D), f32)
    wv_max = jnp.zeros((8, D), f32)
    starts = {r0 // TA: c for c, (r0, _) in enumerate(X_CHUNKS)}
    for u in range(S // TA):
        if u == 0:
            wqkv_copy(1).wait()
        if u + 1 in starts:
            x_copy(starts[u + 1]).wait()
        if u == W_AT:
            wqkv_copy(0).wait()
            wqkv_copy(2).wait()
        if u >= W_AT:
            wv_max = jnp.maximum(wv_max, w_transposes(u - W_AT))
        kmax8 = jnp.maximum(kmax8, k_proj(_wide(xns, slice(u * TA, (u + 1) * TA)), u * TA, TA))
        if u + 1 < S // TA:
            first_ln(u + 1)
    kmx[...] = kmax8
    wv_max = jnp.max(wv_max)
    v_ok = (wv_max >= WV_MIN) & (wv_max <= WV_MAX)

    def layer(li, carry):
        def k_stats():
            kmax = jnp.maximum(jnp.max(kmx[...], axis=0, keepdims=True), 1e-30)
            kc = jnp.broadcast_to(kmax, (128, D)).T
            for h in range(H):
                tmp[0, h * HS:h * HS + DH, :] = kc[h * DH:(h + 1) * DH]
            for o in range(4):
                for d in range(DH):
                    r = o * 128 + d * 8
                    tmp[1, r:r + 8, :] = tmp[0, pl.ds(o * 8 * HS + d, 8, stride=HS), :]
            return jnp.broadcast_to(127.0 / kmax, (8, D))

        def k_limbs(r0, gg, beta8):
            seg = (jax.lax.broadcasted_iota(i32, (8, 128), 1) // DH) % 4
            y = kf[pl.ds(r0, 32), gg * 128:(gg + 1) * 128].reshape(4, 8, 128) \
                * beta8[:, gg * 128:(gg + 1) * 128]
            t0 = _bits(y + MAGIC)
            te = _bits(y + MAGIC / 16) - (t0 << 4)
            t1 = _bits(y + MAGIC * 16)
            y0, ey, y1 = [pltpu.bitcast(a.reshape(32, 128).astype(i8), i32)
                          for a in (t0, te, t1)]

            def rolled(a, k):
                return a if k == 0 else pltpu.roll(a, (DH * k) % 128, 1)
            ry0 = {k: rolled(y0, k) for k in range(-3, 2)}
            rey = {k: rolled(ey, k) for k in range(-1, 3)}
            ry1 = {k: rolled(y1, k) for k in range(0, 4)}
            for r in range(4):
                out = jnp.where(seg < 2,
                                jnp.where(seg == 0, ry0[0 - r], ry0[1 - r]),
                                jnp.where(seg == 2, rey[2 - r], ry1[3 - r]))
                kl[gg * 4 + r, pl.ds(r0, 32), :] = pltpu.bitcast(out, i8)

        def q_limbs(ct, o, k):
            r = o * 128 + k * 32
            q = qT[ct, r:r + 32, :].reshape(4, 8, 128)
            a1 = al[ct, o * 8:(o + 1) * 8, :]
            a256 = a1 * 256.0
            x = (q[0] * a1, q[1] * a256, q[2] * a1, q[3] * a256)
            w0, u, x1, w16 = [_pack_rounded(x, e, (cst[2 * i], cst[2 * i + 1]))
                              for i, (e, _) in enumerate(PACKS)]
            for j, word in enumerate((u, w0 - u, x1, w16 - (w0 << 4))):
                r = (4 * j + k) * QS + o * 8
                qw[ct, r:r + 8, :] = word ^ SIGN_BYTES

        def q_raw(r0):
            return jax.lax.dot_general(pltpu.bitcast(wqT[...], bf16), _wide(xns, pl.ds(r0, 128)),
                                       NT, preferred_element_type=f32)

        beta8 = k_stats()
        bound = jnp.zeros((8, 128), f32)
        for ct in range(NC):
            r0 = ct * 128
            q = q_raw(r0) * tmp[1, 0:D, :]
            qT[ct, 0:D, :] = q
            aq = jnp.abs(q).reshape(4, DH, 8, 128)
            amax = jnp.maximum(jnp.max(aq, axis=1), 1e-30).reshape(H, 128)
            al[ct] = 254.0 / amax
            cs[ct] = amax * (SCALE * LOG2E / (254.0 * 127.0))
            bound = jnp.maximum(bound, jnp.max(jnp.sum(aq, axis=1), axis=0))
            for rb in range(4):
                for gg in range(4):
                    k_limbs(r0 + rb * 32, gg, beta8)

        def vproj(t, _):
            p_c[...] = jnp.zeros(p_c.shape, f32)
            acc_c[...] = jnp.zeros(acc_c.shape, f32)
            l_c[...] = jnp.ones(l_c.shape, f32)
            v_c[2 * PAIRS - 1, S // TK - 1] = jnp.zeros((8, 128), i32)
            for cc in range(TA2 // 128):
                ct = t * (TA2 // 128) + cc
                r0 = pl.multiple_of(ct * 128, 128)
                xn = _wide(xns, pl.ds(r0, 128))
                for o in range(4):
                    rows = slice(o * 128, (o + 1) * 128)
                    wv = pltpu.bitcast(wvT[o * 64:(o + 1) * 64, :], bf16)
                    v = jax.lax.dot_general(wv, xn, NT, preferred_element_type=f32)
                    vT[ct, rows, :] = v.astype(bf16)
                    for k in range(4):
                        q_limbs(ct, o, k)
            return jnp.max(bound)
        bmax = jax.lax.fori_loop(0, S // TA2, vproj, jnp.float32(0))
        safe = (bmax * (SCALE * LOG2E) < SAFE_LOG2) & v_ok

        def o_transpose(r0):
            on = oT[:, pl.ds(_aligned(r0, TS), TS)].T
            for j in range(ND):
                oN[j] = on[:, j * 128:(j + 1) * 128]

        @pl.when(safe)
        def _fast():
            nq = S // TQ
            nk = S // TK
            cq = TQ // 128

            def head_of(g, b):
                return ((g >> 2) << 3) + 4 * b + (g & 3)

            def pv(v, p, acc, s=None):
                never = pltpu.bitcast(acc_c[1, 0:8, 0:128], i32) != 0
                outs = []
                for t in range(cq):
                    vt = v
                    if s is not None and t in (2, 3):
                        dep = s[TIE_ROW:TIE_ROW + 8, (t + 2) * 128:(t + 3) * 128]
                        vt = jnp.where(never, dep, v)
                    outs.append(jnp.dot(pltpu.bitcast(vt, bf16),
                                        p[:, t * 128:(t + 1) * 128].astype(bf16),
                                        preferred_element_type=f32))
                return acc + jnp.concatenate(outs, axis=1)

            def finish(h, q0, acc, ls):
                lsum = jnp.sum(ls, axis=0, keepdims=True)
                r = pl.reciprocal(lsum, approx=True)
                r = r * (2.0 - lsum * r)
                oT[pl.ds(_aligned(h * DH, DH), DH), pl.ds(q0, TQ)] = (acc * r).astype(bf16)

            def body(i, _):
                ph, pq0 = head_of(jnp.maximum(i * PAIRS - 1, 0), 1), (nq - 1) * TQ
                p, acc, pls = p_c[...], acc_c[0], l_c[...]
                pv_last = v_c[2 * PAIRS - 1, nk - 1]
                zero = jnp.zeros((DH, TQ), i32)
                for gi in range(PAIRS):
                    g = i * PAIRS + gi
                    k_c[gi] = pltpu.roll(pltpu.bitcast(kl[g], i32), 64, 1)
                    for b in range(2):
                        h = head_of(g, b)
                        for kc in range(nk):
                            v_c[2 * gi + b, kc] = pltpu.bitcast(
                                vT[kc, pl.ds(_aligned(h * DH, DH), DH), :], i32)
                        for j in range(NC):
                            c_c[2 * gi + b, :, j * 128:(j + 1) * 128] = jnp.broadcast_to(
                                cs[j, pl.ds(h, 1), :], (8, 128))
                    for qt in range(nq):
                        for b in range(2):
                            h = head_of(g, b)
                            n = 2 * gi + b
                            words = jnp.concatenate(
                                [qw[qt * cq + j, pl.ds(h, DH, stride=QS), :] for j in range(cq)],
                                axis=1)
                            w = pltpu.bitcast(jnp.concatenate([words, zero], axis=0), i8)
                            c = c_c[n, :, qt * TQ:(qt + 1) * TQ]
                            ls = None
                            for kc in range(nk):
                                if b == 0:
                                    kk = kl[g, kc * TK:(kc + 1) * TK, :]
                                else:
                                    kk = pltpu.bitcast(
                                        k_c[gi, kc * (TK // 4):(kc + 1) * (TK // 4), :], i8)
                                s = jnp.dot(kk, w, preferred_element_type=i32)
                                if kc == 0:
                                    finish(ph, pq0, pv(pv_last, p, acc, s), pls)
                                    acc = acc_c[1]
                                else:
                                    acc = pv(v_c[n, kc - 1], p, acc, s)
                                p = jnp.exp2(s.astype(f32).reshape(TK // 8, 8, TQ) * c)
                                psum = jnp.sum(p, axis=0)
                                ls = psum if ls is None else ls + psum
                                p = p.reshape(TK, TQ)
                            ph, pq0, pls, pv_last = h, qt * TQ, ls, v_c[n, nk - 1]
                p_c[...] = p
                acc_c[0] = acc
                l_c[...] = pls
                return 0
            jax.lax.fori_loop(0, NG // PAIRS, body, 0)
            o_transpose(0)
            finish(H - 1, (nq - 1) * TQ,
                   pv(v_c[2 * PAIRS - 1, nk - 1], p_c[...], acc_c[0]), l_c[...])

        @pl.when(jnp.logical_not(safe))
        def _slow():
            def qraw(ct, _):
                qT[ct, 0:D, :] = q_raw(pl.multiple_of(ct * 128, 128))
                return 0
            jax.lax.fori_loop(0, NC, qraw, 0)

            def body(i, _):
                h = i // NC
                ct = i % NC
                q0 = pl.multiple_of(ct * 128, 128)
                g0 = pl.multiple_of((h // 8) * 128, 128)
                r0 = pl.multiple_of(h * DH, DH)
                qh = qT[ct, pl.ds(g0 + h % 8, DH, stride=8), :]
                row = jax.lax.broadcasted_iota(i32, (128, 128), 0)
                w = jnp.where(row // DH == h % 8, jnp.concatenate([qh] * 8, axis=0), 0.0)
                kb = kf[:, pl.ds(g0, 128)].astype(bf16)
                s = jnp.dot(kb, w.astype(bf16), preferred_element_type=f32) * SCALE
                m = jnp.max(s, axis=0, keepdims=True)
                p = jnp.exp(s - m)
                lsum = jnp.sum(p, axis=0, keepdims=True)
                acc = jnp.dot(_wide(vT, pl.ds(r0, DH)), p.astype(bf16),
                              preferred_element_type=f32)
                oT[pl.ds(r0, DH), pl.ds(q0, 128)] = (acc / lsum).astype(bf16)
                return 0
            jax.lax.fori_loop(0, H * NC, body, 0)
            o_transpose(0)

        def ffn(t, last):
            ns = TM // TS
            rs = [pl.multiple_of(t * TM + u * TS, TS) for u in range(ns)]
            b1 = b1f[...]
            b2 = b2f[...]
            x0 = [(xs if last else xb)[pl.ds(r, TS), :].astype(f32) for r in rs]
            x1 = [x0[0] + jnp.dot(_wide(oN), wo[...], preferred_element_type=f32)]
            x1 += [x + jax.lax.dot_general(
                oT[:, pl.ds(r, TS)], wo[...], TN, preferred_element_type=f32)
                for r, x in zip(rs[1:], x0[1:])]
            o_transpose(jnp.minimum(t + 1, S // TM - 1) * TM)
            hh = [_gelu(jnp.dot(_layernorm(x).astype(bf16), w1[...],
                                preferred_element_type=f32) + b1).astype(bf16) for x in x1]
            x2 = []
            for u, (r, x, g) in enumerate(zip(rs, x1, hh)):
                x = x + jnp.dot(g, w2[...], preferred_element_type=f32) + b2
                if last:
                    xb[pl.ds(r, TS), :] = x.astype(bf16)
                    out_copy(t * ns + u).start()
                else:
                    xs[pl.ds(r, TS), :] = x
                    x2.append(x)
            if not last:
                km = kmx[...]
                for r, x in zip(rs, x2):
                    km = jnp.maximum(km, k_proj(ln_store(x, r, TS), r, TS))
                kmx[...] = km
            return 0

        @pl.when(li == 0)
        def _():
            for cp in late:
                cp.wait()
            b1f[...] = b1v[...].astype(f32).reshape(1, F)
            b2f[...] = b2v[...].astype(f32).reshape(1, D)

        @pl.when(li < N_LAYERS - 1)
        def _():
            kmx[...] = jnp.zeros(kmx.shape, f32)
            jax.lax.fori_loop(0, S // TM, lambda t, _: ffn(t, False), 0)

        @pl.when(li == N_LAYERS - 1)
        def _():
            jax.lax.fori_loop(0, S // TM, lambda t, _: ffn(t, True), 0)
        return carry

    jax.lax.fori_loop(0, N_LAYERS, layer, 0)
    for u in range(S // TS):
        out_copy(u).wait()


@jax.jit
def pallas_interleave_layers__mha_block__dense_activation_gelu__prompt_kernel(
    A_x: jax.Array,
    A_wqkv: jax.Array,
    A_wo: jax.Array,
    B_x: jax.Array,
    B_w1: jax.Array,
    B_b1: jax.Array,
    B_w2: jax.Array,
    B_b2: jax.Array,
):
    del B_x
    hbm = pl.BlockSpec(memory_space=pl.ANY)
    out = pl.pallas_call(
        _kernel,
        out_shape=jax.ShapeDtypeStruct((S, D), A_x.dtype),
        in_specs=[hbm] * 7,
        out_specs=hbm,
        scratch_shapes=[
            pltpu.VMEM((S, D), bf16),
            pltpu.VMEM((3, D, D), bf16),
            pltpu.VMEM((D, D), bf16),
            pltpu.VMEM((D, F), bf16),
            pltpu.VMEM((F, D), bf16),
            pltpu.SemaphoreType.DMA((NX + 5,)),
            pltpu.VMEM((S, D), f32),
            pltpu.VMEM((ND, S, 128), bf16),
            pltpu.VMEM((D // 2, D), i32),
            pltpu.VMEM((D // 2, D), i32),
            pltpu.VMEM((ND, (H + 1) * HS, 128), f32),
            pltpu.VMEM((S, D), f32),
            pltpu.VMEM((8, D), f32),
            pltpu.VMEM((NC, D + 8, 128), f32),
            pltpu.VMEM((NC, D, 128), bf16),
            pltpu.VMEM((NG, S, 128), i8),
            pltpu.VMEM((NC, (DH + 1) * QS, 128), i32),
            pltpu.VMEM((NC, H, 128), f32),
            pltpu.VMEM((NC, H, 128), f32),
            pltpu.VMEM((D, S), bf16),
            pltpu.VMEM((ND, TS, 128), bf16),
            pltpu.VMEM((TK, TQ), f32),
            pltpu.VMEM((2, DH, TQ), f32),
            pltpu.VMEM((8, TQ), f32),
            pltpu.VMEM((PAIRS, S // 4, 128), i32),
            pltpu.VMEM((2 * PAIRS, NC, 8, 128), i32),
            pltpu.VMEM((2 * PAIRS, 8, S), f32),
            pltpu.VMEM((8, 8, 128), f32),
            pltpu.VMEM((F,), bf16),
            pltpu.VMEM((D,), bf16),
            pltpu.VMEM((1, F), f32),
            pltpu.VMEM((1, D), f32),
        ],
        compiler_params=pltpu.CompilerParams(vmem_limit_bytes=100 * 1024 * 1024),
    )(A_x.reshape(S, D), A_wqkv, A_wo, B_w1, B_b1, B_w2, B_b2)
    return out.reshape(1, S, D)
```

```python
import jax
import jax.numpy as jnp
import jax.experimental.pallas as pl
import jax.experimental.pallas.tpu as pltpu

S, D, H, DH, F = 2048, 512, 32, 16, 1792
N_LAYERS = 2
EPS = 1e-5
LOG2E = 1.4426950408889634
SCALE = DH ** -0.5
MAGIC = 12582912.0

SIGN_BYTES = 0x80808080 - 2 ** 32

NG = H // 2
NC = S // 128
ND = D // 128
X_CHUNKS = ((0, 256), (256, 256), (512, 768), (1280, 768))
NX = len(X_CHUNKS)
TA = 256
W_AT = 4
TA2 = 1024
TM = 256
TS = 128
TQ = 1024
PAIRS = 2
TK = 128
TIE_ROW = 40
HS = 24
QS = 40

SAFE_LOG2 = 64.0
WV_MIN, WV_MAX = 2.0 ** -20, 2.0 ** 20

bf16 = jnp.bfloat16
f32 = jnp.float32
i32 = jnp.int32
i8 = jnp.int8
NT = (((1,), (1,)), ((), ()))
TN = (((0,), (0,)), ((), ()))


def _layernorm(x):
    m = jnp.mean(x, axis=-1, keepdims=True)
    xc = x - m
    v = jnp.mean(xc * xc, axis=-1, keepdims=True)
    return xc * jax.lax.rsqrt(v + EPS)


def _gelu(x):
    c = 0.7978845608028654
    return 0.5 * x * (1.0 + jnp.tanh(c * (x + 0.044715 * (x * x * x))))


def _bits(t):
    return pltpu.bitcast(t, i32)


PACKS = ((0, 256), (1, 128), (4, 128), (-4, 16 * 256 + 128))
BIG = 2.0 ** 31 + 2.0 ** 21


def _pack_consts(e, off):
    return [(BIG - 2.0 ** 23 - 257 * off - extra) * 2.0 ** e
            for extra in (0, 2 ** 16 - ((150 + e) << 7))]


def _pack_rounded(x, e, sub):
    def pair(lo, hi256, c):
        return _bits(((hi256 + BIG * 2.0 ** e) - c) + lo)
    return pair(x[0], x[1], sub[0]) + (pair(x[2], x[3], sub[1]) << 16)


def _wide(ref, rows=slice(None)):
    return jnp.concatenate([ref[j, rows, :] for j in range(ref.shape[0])], axis=1)


def _aligned(i, n):
    return i if isinstance(i, int) else pl.multiple_of(i, n)


def _kernel(x_hbm, wqkv_hbm, wo_hbm, w1_hbm, b1_hbm, w2_hbm, b2_hbm, o_hbm,
            xb, wqkv, wo, w1, w2, sems,
            xs, xns, wqT, wvT, tmp, kf, kmx, qT, vT, kl, qw, cs, al, oT, oN,
            p_c, acc_c, l_c, k_c, v_c, c_c, cst, b1v, b2v, b1f, b2f):

    def x_copy(c):
        r0, n = X_CHUNKS[c]
        return pltpu.make_async_copy(x_hbm.at[pl.ds(r0, n), :], xb.at[pl.ds(r0, n), :],
                                     sems.at[c])

    def wqkv_copy(j):
        return pltpu.make_async_copy(wqkv_hbm.at[:, pl.ds(j * D, D)], wqkv.at[j],
                                     sems.at[NX + j])

    late = [pltpu.make_async_copy(src, dst, sems.at[NX + 3]) for src, dst in
            ((wo_hbm, wo), (w1_hbm, w1), (w2_hbm, w2), (b1_hbm, b1v), (b2_hbm, b2v))]

    def out_copy(u):
        r0 = _aligned(u * TS, TS)
        return pltpu.make_async_copy(xb.at[pl.ds(r0, TS), :], o_hbm.at[pl.ds(r0, TS), :],
                                     sems.at[NX + 4])

    x_copy(0).start()
    wqkv_copy(1).start()
    for c in range(1, NX):
        x_copy(c).start()
    wqkv_copy(0).start()
    wqkv_copy(2).start()

    for i, (e, off) in enumerate(PACKS):
        for j, c in enumerate(_pack_consts(e, off)):
            cst[2 * i + j] = jnp.full((8, 128), c, f32)

    for ct in range(NC):
        for j in range(DH):
            qw[ct, j * QS + H:(j + 1) * QS, :] = jnp.zeros((QS - H, 128), i32)
        qw[ct, DH * QS:, :] = jnp.zeros((QS, 128), i32)
        qT[ct, D:, :] = jnp.zeros((8, 128), f32)
    for j in range(ND):
        for h in range(H):
            tmp[j, h * HS + DH:(h + 1) * HS, :] = jnp.zeros((HS - DH, 128), f32)
        tmp[j, H * HS:, :] = jnp.zeros((HS, 128), f32)

    def ln_store(x, r0, n):
        xn = _layernorm(x).astype(bf16)
        for j in range(ND):
            xns[j, pl.ds(r0, n), :] = xn[:, j * 128:(j + 1) * 128]
        return xn

    def k_proj(xn, r0, n):
        k = jnp.dot(xn, wqkv[1], preferred_element_type=f32)
        kf[pl.ds(r0, n), :] = k
        return jnp.max(jnp.abs(k).reshape(n // 8, 8, D), axis=0)

    def first_ln(u):
        ln_store(xb[u * TA:(u + 1) * TA, :].astype(f32), u * TA, TA)

    def wq_transpose(j):
        cols = slice(j * 128, (j + 1) * 128)
        wq_t = wqkv[0, cols, :].T.astype(f32)
        for h in range(H):
            tmp[j, h * HS:h * HS + DH, :] = wq_t[h * DH:(h + 1) * DH]
        for o in range(4):
            for d2 in range(DH // 2):
                r = o * 64 + d2 * 8
                wqT[r:r + 8, cols] = pltpu.bitcast(jnp.concatenate(
                    [tmp[j, pl.ds(o * 8 * HS + 2 * d2 + e, 8, stride=HS), :]
                     for e in range(2)], axis=0).astype(bf16), i32)

    x_copy(0).wait()
    first_ln(0)
    kmax8 = jnp.zeros((8, D), f32)
    starts = {r0 // TA: c for c, (r0, _) in enumerate(X_CHUNKS)}
    for u in range(S // TA):
        if u == 0:
            wqkv_copy(1).wait()
        if u + 1 in starts:
            x_copy(starts[u + 1]).wait()
        if u == W_AT:
            wqkv_copy(0).wait()
            for cp in late:
                cp.start()
        if u >= W_AT:
            wq_transpose(u - W_AT)
        kmax8 = jnp.maximum(kmax8, k_proj(_wide(xns, slice(u * TA, (u + 1) * TA)), u * TA, TA))
        if u + 1 < S // TA:
            first_ln(u + 1)
    kmx[...] = kmax8
    wqkv_copy(2).wait()

    def layer(li, carry):
        def k_stats():
            kmax = jnp.maximum(jnp.max(kmx[...], axis=0, keepdims=True), 1e-30)
            kc = jnp.broadcast_to(kmax, (128, D)).T
            for h in range(H):
                tmp[0, h * HS:h * HS + DH, :] = kc[h * DH:(h + 1) * DH]
            for o in range(4):
                for d in range(DH):
                    r = o * 128 + d * 8
                    tmp[1, r:r + 8, :] = tmp[0, pl.ds(o * 8 * HS + d, 8, stride=HS), :]
            return jnp.broadcast_to(127.0 / kmax, (8, D))

        def k_limbs(r0, gg, beta8):
            seg = (jax.lax.broadcasted_iota(i32, (8, 128), 1) // DH) % 4
            y = kf[pl.ds(r0, 32), gg * 128:(gg + 1) * 128].reshape(4, 8, 128) \
                * beta8[:, gg * 128:(gg + 1) * 128]
            t0 = _bits(y + MAGIC)
            te = _bits(y + MAGIC / 16) - (t0 << 4)
            t1 = _bits(y + MAGIC * 16)
            y0, ey, y1 = [pltpu.bitcast(a.reshape(32, 128).astype(i8), i32)
                          for a in (t0, te, t1)]

            def rolled(a, k):
                return a if k == 0 else pltpu.roll(a, (DH * k) % 128, 1)
            ry0 = {k: rolled(y0, k) for k in range(-3, 2)}
            rey = {k: rolled(ey, k) for k in range(-1, 3)}
            ry1 = {k: rolled(y1, k) for k in range(0, 4)}
            for r in range(4):
                out = jnp.where(seg < 2,
                                jnp.where(seg == 0, ry0[0 - r], ry0[1 - r]),
                                jnp.where(seg == 2, rey[2 - r], ry1[3 - r]))
                kl[gg * 4 + r, pl.ds(r0, 32), :] = pltpu.bitcast(out, i8)

        def q_limbs(ct, o, k):
            r = o * 128 + k * 32
            q = qT[ct, r:r + 32, :].reshape(4, 8, 128)
            a1 = al[ct, o * 8:(o + 1) * 8, :]
            a256 = a1 * 256.0
            x = (q[0] * a1, q[1] * a256, q[2] * a1, q[3] * a256)
            w0, u, x1, w16 = [_pack_rounded(x, e, (cst[2 * i], cst[2 * i + 1]))
                              for i, (e, _) in enumerate(PACKS)]
            for j, word in enumerate((u, w0 - u, x1, w16 - (w0 << 4))):
                r = (4 * j + k) * QS + o * 8
                qw[ct, r:r + 8, :] = word ^ SIGN_BYTES

        def q_raw(r0):
            return jax.lax.dot_general(pltpu.bitcast(wqT[...], bf16), _wide(xns, pl.ds(r0, 128)),
                                       NT, preferred_element_type=f32)

        beta8 = k_stats()
        wvT[...] = pltpu.bitcast(wqkv[2].T, i32)
        wv_max = jnp.max(jnp.abs(wqkv[2].astype(f32)))
        v_ok = (wv_max >= WV_MIN) & (wv_max <= WV_MAX)
        bound = jnp.zeros((8, 128), f32)
        for ct in range(NC):
            r0 = ct * 128
            q = q_raw(r0) * tmp[1, 0:D, :]
            qT[ct, 0:D, :] = q
            aq = jnp.abs(q).reshape(4, DH, 8, 128)
            amax = jnp.maximum(jnp.max(aq, axis=1), 1e-30).reshape(H, 128)
            al[ct] = 254.0 / amax
            cs[ct] = amax * (SCALE * LOG2E / (254.0 * 127.0))
            bound = jnp.maximum(bound, jnp.max(jnp.sum(aq, axis=1), axis=0))
            for rb in range(4):
                for gg in range(4):
                    k_limbs(r0 + rb * 32, gg, beta8)

        def vproj(t, _):
            p_c[...] = jnp.zeros(p_c.shape, f32)
            acc_c[...] = jnp.zeros(acc_c.shape, f32)
            l_c[...] = jnp.ones(l_c.shape, f32)
            v_c[2 * PAIRS - 1, S // TK - 1] = jnp.zeros((8, 128), i32)
            for cc in range(TA2 // 128):
                ct = t * (TA2 // 128) + cc
                r0 = pl.multiple_of(ct * 128, 128)
                xn = _wide(xns, pl.ds(r0, 128))
                for o in range(4):
                    rows = slice(o * 128, (o + 1) * 128)
                    wv = pltpu.bitcast(wvT[o * 64:(o + 1) * 64, :], bf16)
                    v = jax.lax.dot_general(wv, xn, NT, preferred_element_type=f32)
                    vT[ct, rows, :] = v.astype(bf16)
                    for k in range(4):
                        q_limbs(ct, o, k)
            return jnp.max(bound)
        bmax = jax.lax.fori_loop(0, S // TA2, vproj, jnp.float32(0))
        safe = (bmax * (SCALE * LOG2E) < SAFE_LOG2) & v_ok

        def o_transpose(r0):
            on = oT[:, pl.ds(_aligned(r0, TS), TS)].T
            for j in range(ND):
                oN[j] = on[:, j * 128:(j + 1) * 128]

        @pl.when(safe)
        def _fast():
            nq = S // TQ
            nk = S // TK
            cq = TQ // 128

            def head_of(g, b):
                return ((g >> 2) << 3) + 4 * b + (g & 3)

            def pv(v, p, acc, s=None):
                never = pltpu.bitcast(acc_c[1, 0:8, 0:128], i32) != 0
                outs = []
                for t in range(cq):
                    vt = v
                    if s is not None and t in (2, 3):
                        dep = s[TIE_ROW:TIE_ROW + 8, (t + 2) * 128:(t + 3) * 128]
                        vt = jnp.where(never, dep, v)
                    outs.append(jnp.dot(pltpu.bitcast(vt, bf16),
                                        p[:, t * 128:(t + 1) * 128].astype(bf16),
                                        preferred_element_type=f32))
                return acc + jnp.concatenate(outs, axis=1)

            def finish(h, q0, acc, ls):
                lsum = jnp.sum(ls, axis=0, keepdims=True)
                r = pl.reciprocal(lsum, approx=True)
                r = r * (2.0 - lsum * r)
                oT[pl.ds(_aligned(h * DH, DH), DH), pl.ds(q0, TQ)] = (acc * r).astype(bf16)

            def body(i, _):
                ph, pq0 = head_of(jnp.maximum(i * PAIRS - 1, 0), 1), (nq - 1) * TQ
                p, acc, pls = p_c[...], acc_c[0], l_c[...]
                pv_last = v_c[2 * PAIRS - 1, nk - 1]
                zero = jnp.zeros((DH, TQ), i32)
                for gi in range(PAIRS):
                    g = i * PAIRS + gi
                    k_c[gi] = pltpu.roll(pltpu.bitcast(kl[g], i32), 64, 1)
                    for b in range(2):
                        h = head_of(g, b)
                        for kc in range(nk):
                            v_c[2 * gi + b, kc] = pltpu.bitcast(
                                vT[kc, pl.ds(_aligned(h * DH, DH), DH), :], i32)
                        for j in range(NC):
                            c_c[2 * gi + b, :, j * 128:(j + 1) * 128] = jnp.broadcast_to(
                                cs[j, pl.ds(h, 1), :], (8, 128))
                    for qt in range(nq):
                        for b in range(2):
                            h = head_of(g, b)
                            n = 2 * gi + b
                            words = jnp.concatenate(
                                [qw[qt * cq + j, pl.ds(h, DH, stride=QS), :] for j in range(cq)],
                                axis=1)
                            w = pltpu.bitcast(jnp.concatenate([words, zero], axis=0), i8)
                            c = c_c[n, :, qt * TQ:(qt + 1) * TQ]
                            ls = None
                            for kc in range(nk):
                                if b == 0:
                                    kk = kl[g, kc * TK:(kc + 1) * TK, :]
                                else:
                                    kk = pltpu.bitcast(
                                        k_c[gi, kc * (TK // 4):(kc + 1) * (TK // 4), :], i8)
                                s = jnp.dot(kk, w, preferred_element_type=i32)
                                if kc == 0:
                                    finish(ph, pq0, pv(pv_last, p, acc, s), pls)
                                    acc = acc_c[1]
                                else:
                                    acc = pv(v_c[n, kc - 1], p, acc, s)
                                p = jnp.exp2(s.astype(f32).reshape(TK // 8, 8, TQ) * c)
                                psum = jnp.sum(p, axis=0)
                                ls = psum if ls is None else ls + psum
                                p = p.reshape(TK, TQ)
                            ph, pq0, pls, pv_last = h, qt * TQ, ls, v_c[n, nk - 1]
                p_c[...] = p
                acc_c[0] = acc
                l_c[...] = pls
                return 0
            jax.lax.fori_loop(0, NG // PAIRS, body, 0)
            o_transpose(0)
            finish(H - 1, (nq - 1) * TQ,
                   pv(v_c[2 * PAIRS - 1, nk - 1], p_c[...], acc_c[0]), l_c[...])

        @pl.when(jnp.logical_not(safe))
        def _slow():
            def qraw(ct, _):
                qT[ct, 0:D, :] = q_raw(pl.multiple_of(ct * 128, 128))
                return 0
            jax.lax.fori_loop(0, NC, qraw, 0)

            def body(i, _):
                h = i // NC
                ct = i % NC
                q0 = pl.multiple_of(ct * 128, 128)
                g0 = pl.multiple_of((h // 8) * 128, 128)
                r0 = pl.multiple_of(h * DH, DH)
                qh = qT[ct, pl.ds(g0 + h % 8, DH, stride=8), :]
                row = jax.lax.broadcasted_iota(i32, (128, 128), 0)
                w = jnp.where(row // DH == h % 8, jnp.concatenate([qh] * 8, axis=0), 0.0)
                kb = kf[:, pl.ds(g0, 128)].astype(bf16)
                s = jnp.dot(kb, w.astype(bf16), preferred_element_type=f32) * SCALE
                m = jnp.max(s, axis=0, keepdims=True)
                p = jnp.exp(s - m)
                lsum = jnp.sum(p, axis=0, keepdims=True)
                acc = jnp.dot(_wide(vT, pl.ds(r0, DH)), p.astype(bf16),
                              preferred_element_type=f32)
                oT[pl.ds(r0, DH), pl.ds(q0, 128)] = (acc / lsum).astype(bf16)
                return 0
            jax.lax.fori_loop(0, H * NC, body, 0)
            o_transpose(0)

        def ffn(t, last):
            ns = TM // TS
            rs = [pl.multiple_of(t * TM + u * TS, TS) for u in range(ns)]
            b1 = b1f[...]
            b2 = b2f[...]
            x0 = [(xs if last else xb)[pl.ds(r, TS), :].astype(f32) for r in rs]
            x1 = [x0[0] + jnp.dot(_wide(oN), wo[...], preferred_element_type=f32)]
            x1 += [x + jax.lax.dot_general(
                oT[:, pl.ds(r, TS)], wo[...], TN, preferred_element_type=f32)
                for r, x in zip(rs[1:], x0[1:])]
            o_transpose(jnp.minimum(t + 1, S // TM - 1) * TM)
            hh = [_gelu(jnp.dot(_layernorm(x).astype(bf16), w1[...],
                                preferred_element_type=f32) + b1).astype(bf16) for x in x1]
            x2 = []
            for u, (r, x, g) in enumerate(zip(rs, x1, hh)):
                x = x + jnp.dot(g, w2[...], preferred_element_type=f32) + b2
                if last:
                    xb[pl.ds(r, TS), :] = x.astype(bf16)
                    out_copy(t * ns + u).start()
                else:
                    xs[pl.ds(r, TS), :] = x
                    x2.append(x)
            if not last:
                km = kmx[...]
                for r, x in zip(rs, x2):
                    km = jnp.maximum(km, k_proj(ln_store(x, r, TS), r, TS))
                kmx[...] = km
            return 0

        @pl.when(li == 0)
        def _():
            for cp in late:
                cp.wait()
            b1f[...] = b1v[...].astype(f32).reshape(1, F)
            b2f[...] = b2v[...].astype(f32).reshape(1, D)

        @pl.when(li < N_LAYERS - 1)
        def _():
            kmx[...] = jnp.zeros(kmx.shape, f32)
            jax.lax.fori_loop(0, S // TM, lambda t, _: ffn(t, False), 0)

        @pl.when(li == N_LAYERS - 1)
        def _():
            jax.lax.fori_loop(0, S // TM, lambda t, _: ffn(t, True), 0)
        return carry

    jax.lax.fori_loop(0, N_LAYERS, layer, 0)
    for u in range(S // TS):
        out_copy(u).wait()


@jax.jit
def pallas_interleave_layers__mha_block__dense_activation_gelu__prompt_kernel(
    A_x: jax.Array,
    A_wqkv: jax.Array,
    A_wo: jax.Array,
    B_x: jax.Array,
    B_w1: jax.Array,
    B_b1: jax.Array,
    B_w2: jax.Array,
    B_b2: jax.Array,
):
    del B_x
    hbm = pl.BlockSpec(memory_space=pl.ANY)
    out = pl.pallas_call(
        _kernel,
        out_shape=jax.ShapeDtypeStruct((S, D), A_x.dtype),
        in_specs=[hbm] * 7,
        out_specs=hbm,
        scratch_shapes=[
            pltpu.VMEM((S, D), bf16),
            pltpu.VMEM((3, D, D), bf16),
            pltpu.VMEM((D, D), bf16),
            pltpu.VMEM((D, F), bf16),
            pltpu.VMEM((F, D), bf16),
            pltpu.SemaphoreType.DMA((NX + 5,)),
            pltpu.VMEM((S, D), f32),
            pltpu.VMEM((ND, S, 128), bf16),
            pltpu.VMEM((D // 2, D), i32),
            pltpu.VMEM((D // 2, D), i32),
            pltpu.VMEM((ND, (H + 1) * HS, 128), f32),
            pltpu.VMEM((S, D), f32),
            pltpu.VMEM((8, D), f32),
            pltpu.VMEM((NC, D + 8, 128), f32),
            pltpu.VMEM((NC, D, 128), bf16),
            pltpu.VMEM((NG, S, 128), i8),
            pltpu.VMEM((NC, (DH + 1) * QS, 128), i32),
            pltpu.VMEM((NC, H, 128), f32),
            pltpu.VMEM((NC, H, 128), f32),
            pltpu.VMEM((D, S), bf16),
            pltpu.VMEM((ND, TS, 128), bf16),
            pltpu.VMEM((TK, TQ), f32),
            pltpu.VMEM((2, DH, TQ), f32),
            pltpu.VMEM((8, TQ), f32),
            pltpu.VMEM((PAIRS, S // 4, 128), i32),
            pltpu.VMEM((2 * PAIRS, NC, 8, 128), i32),
            pltpu.VMEM((2 * PAIRS, 8, S), f32),
            pltpu.VMEM((8, 8, 128), f32),
            pltpu.VMEM((F,), bf16),
            pltpu.VMEM((D,), bf16),
            pltpu.VMEM((1, F), f32),
            pltpu.VMEM((1, D), f32),
        ],
        compiler_params=pltpu.CompilerParams(vmem_limit_bytes=100 * 1024 * 1024),
    )(A_x.reshape(S, D), A_wqkv, A_wo, B_w1, B_b1, B_w2, B_b2)
    return out.reshape(1, S, D)
```
